```python
import jax
import jax.numpy as jnp

def _softmax(x, axis=-1):
    return jax.nn.softmax(x, axis=axis)
def _gelu(x):
    return jax.nn.gelu(x, approximate=True)
def _silu(x):
    return jax.nn.silu(x)
def _sigmoid(x):
    return jax.nn.sigmoid(x)
def _layernorm(x, axis=-1, eps=1e-5):
    m = jnp.mean(x, axis=axis, keepdims=True)
    v = jnp.var(x, axis=axis, keepdims=True)
    return (x - m) / jnp.sqrt(v + eps)
def _scatter_add(tgt, idx, src, axis=0):
    return tgt.at[idx].add(src)
def _segment_sum(src, seg, n):
    return jax.ops.segment_sum(src, seg, n)
class _Rng:
    def __init__(self, key):
        self._k = key
    def _next(self):
        self._k, sub = jax.random.split(self._k)
        return sub
    def normal(self, shape):
        return jax.random.normal(self._next(), shape, dtype=jnp.bfloat16)
    def randint(self, lo, hi, shape):
        return jax.random.randint(self._next(), shape, lo, hi, dtype=jnp.int32)
    def uniform(self, shape, lo=0.0, hi=1.0):
        return jax.random.uniform(self._next(), shape, jnp.bfloat16, lo, hi)
    def permutation(self, n):
        return jax.random.permutation(self._next(), n)


kernel_name = 'sequential_preLN__mha_block_cached__mixer_channel_mlp__decode'

def _fwd_setup_inputs():
    _rng = _Rng(jax.random.key(int.from_bytes(__import__("os").urandom(4), "little")))
    _w = (lambda a: (lambda t: t.astype(jnp.bfloat16) if jnp.issubdtype(t.dtype, jnp.floating) else t)(jnp.asarray(a)))
    def _A_setup():
        B, Sq, D = 2, 1, 512
        H, Sk, Dh = 32, 8192, 128
        return {
            "x": _w((lambda *s: _rng.normal(s) * 0.05)(B, Sq, D)),
            "k_cache": _w((lambda *s: _rng.normal(s) * 0.05)(B, H, Sk, Dh)),
            "v_cache": _w((lambda *s: _rng.normal(s) * 0.05)(B, H, Sk, Dh)),
            "wq": _w((lambda *s: _rng.normal(s) * 0.05)(D, H * Dh) * (D ** -0.5)),
            "wo": _w((lambda *s: _rng.normal(s) * 0.05)(H * Dh, D) * ((H * Dh) ** -0.5)),
        }
    _A_in = _A_setup()

    def _B_setup():
        B, S, D, F = 2, 1, 512, 1792
        return {
            "x": _w((lambda *s: _rng.normal(s) * 0.05)(B, S, D)),
            "w1": _w((lambda *s: _rng.normal(s) * 0.05)(D, F) * (D ** -0.5)),
            "b1": _w((lambda *s: _rng.normal(s) * 0.05)(F)),
            "w2": _w((lambda *s: _rng.normal(s) * 0.05)(F, D) * (F ** -0.5)),
            "b2": _w((lambda *s: _rng.normal(s) * 0.05)(D)),
        }
    _B_in = _B_setup()

    return {
        "A_x": _A_in["x"],
        "A_k_cache": _A_in["k_cache"],
        "A_v_cache": _A_in["v_cache"],
        "A_wq": _A_in["wq"],
        "A_wo": _A_in["wo"],
        "B_x": _B_in["x"],
        "B_w1": _B_in["w1"],
        "B_b1": _B_in["b1"],
        "B_w2": _B_in["w2"],
        "B_b2": _B_in["b2"],
    }

def _fwd_reference(A_x, A_k_cache, A_v_cache, A_wq, A_wo, B_x, B_w1, B_b1, B_w2, B_b2):
    def _A_ref(x, k_cache, v_cache, wq, wo):
        B, Sq, D = x.shape
        H, Dh = 32, 128
        q = (lambda x, *d: x.transpose(*d))((x @ wq).reshape(B, Sq, H, Dh), 0, 2, 1, 3)
        scores = jnp.einsum("bhqd,bhkd->bhqk", q, k_cache) * (Dh ** -0.5)
        p = _softmax(scores, axis=-1)
        o = jnp.einsum("bhqk,bhkd->bhqd", p, v_cache)
        return (lambda x, *d: x.transpose(*d))(o, 0, 2, 1, 3).reshape(B, Sq, H * Dh) @ wo

    def _B_ref(x, w1, b1, w2, b2):
        y = _layernorm(x, axis=-1)
        h = _gelu(jnp.einsum("bsd,df->bsf", y, w1) + b1)
        return jnp.einsum("bsf,fd->bsd", h, w2) + b2

    x = A_x
    h = x + _A_ref(_layernorm(x, axis=-1), A_k_cache, A_v_cache, A_wq, A_wo)
    h2 = h + _B_ref(_layernorm(h, axis=-1), B_w1, B_b1, B_w2, B_b2)
    return h2


def setup_inputs():
    _inp = _fwd_setup_inputs()
    _gk = jax.random.fold_in(jax.random.key(int.from_bytes(__import__("os").urandom(4), "little")), 2**31 - 1)
    _shapes = [[2, 1, 512]]
    _dtypes = ['bfloat16']
    _gks = jax.random.split(_gk, len(_shapes))
    _gs = [jax.random.normal(k, s, dtype=jnp.dtype(d)) * 0.05 for k, s, d in zip(_gks, _shapes, _dtypes)]
    _inp["grad_out"] = _gs[0]
    return _inp

def reference(A_x, A_k_cache, A_v_cache, A_wq, A_wo, B_w1, B_b1, B_w2, B_b2, B_x, grad_out):
    _const = dict(B_x=B_x)
    def _f(*_d):
        return _fwd_reference(**{'A_x': _d[0], 'A_k_cache': _d[1], 'A_v_cache': _d[2], 'A_wq': _d[3], 'A_wo': _d[4], 'B_w1': _d[5], 'B_b1': _d[6], 'B_w2': _d[7], 'B_b2': _d[8], **_const})
    _out, _vjp = jax.vjp(_f, A_x, A_k_cache, A_v_cache, A_wq, A_wo, B_w1, B_b1, B_w2, B_b2)
    _grads = _vjp(grad_out)
    _out0 = jnp.asarray(_out)
    return (_out0, *[jnp.asarray(_g) for _g in _grads])
```

```python
import jax
import jax.numpy as jnp
from jax import lax
import jax.experimental.pallas as pl
import jax.experimental.pallas.tpu as pltpu

F32 = jnp.float32
BF16 = jnp.bfloat16

B, H, S, DH = 2, 32, 8192, 128
D, FF = 512, 1792
HD = H * DH
NHEAD = B * H
NQUAD = NHEAD // 4
QPB = H // 4
SROWS = S // 2
PART = SROWS // 2
STEP = SROWS // 4
NSITE = 2 * NHEAD
AHEAD = 3
NVSLOT = QPB + 1
DVSLOT = NVSLOT
NKSLOT = 3
RROWS = 16
WROWS = 64
CH = 256
RP = 16
SCALE = DH ** -0.5
EPS = 1e-5
GELU_C = 0.7978845608028654
GELU_A = 0.044715

NT = (((1,), (1,)), ((), ()))
TN = (((0,), (0,)), ((), ()))


def _dot(a, b):
    return jnp.dot(a, b, preferred_element_type=F32)


def _dot_nt(a, b):
    return lax.dot_general(a, b, NT, preferred_element_type=F32)


def _dot_tn(a, b):
    return lax.dot_general(a, b, TN, preferred_element_type=F32)


def _ln(x):
    mu = jnp.mean(x, axis=-1, keepdims=True)
    xc = x - mu
    var = jnp.mean(xc * xc, axis=-1, keepdims=True)
    rstd = lax.rsqrt(var + EPS)
    return xc * rstd, rstd


def _ln_bwd(dy, y, rstd):
    m1 = jnp.mean(dy, axis=-1, keepdims=True)
    m2 = jnp.mean(dy * y, axis=-1, keepdims=True)
    return (dy - m1 - y * m2) * rstd


def _pad_rows(x2):
    r = lax.broadcasted_iota(jnp.int32, (RP, x2.shape[1]), 0)
    return jnp.where(r == 0, x2[0:1], jnp.where(r == 1, x2[1:2], 0.0))


def _get_row(ref, b, lanes):
    blk = ref[0:8, lanes]
    return jnp.where(b == 0, blk[0:1], blk[1:2])


def _set_row(ref, b, lanes, val8):
    r = lax.broadcasted_iota(jnp.int32, val8.shape, 0)
    ref[0:8, lanes] = jnp.where(r == b, val8, ref[0:8, lanes])


def _outer_tiles(col, row):
    tiles = [col * row[:, j * DH:(j + 1) * DH] for j in range(row.shape[1] // DH)]
    return jnp.concatenate(tiles, axis=1).astype(BF16).T


def _ads(start, size, align):
    return pl.ds(pl.multiple_of(start, align), size)


def _loop(n, body, unroll):
    def wrapped(i, c):
        body(i)
        return c
    lax.fori_loop(0, n, wrapped, 0, unroll=unroll)


def _kernel(x_hbm, k_hbm, v_hbm, wq_hbm, wo_hbm, w1_hbm, b1_hbm, w2_hbm, b2_hbm, go_hbm,
            out_hbm, dx_hbm, dk_hbm, dv_hbm, dwq_hbm, dwo_hbm, dw1_hbm, db1_hbm, dw2_hbm, db2_hbm,
            kbuf, vbuf, wq, wo, w1, w2, dwq, dwo, dw1, dw2,
            x_s, go_s, b1_s, b2_s, out_s, dx_s, db1_s, db2_s,
            rows_all, m_all, acc_s, ksum_s, ml_s, att_s, cols, q_all, o_all, dq_all, xn_all, h_all, y_all, dh_all,
            g_all, da_all, dg_all,
            ksem, vsem, wsem, isem, osem):
    copy = pltpu.make_async_copy

    def kv_refs(n):
        quad = n // 4
        rows = _ads((n % 4) * STEP, STEP, STEP)
        slot = n % NKSLOT
        return (k_hbm.at[quad, :, rows], kbuf.at[slot], ksem.at[slot],
                v_hbm.at[quad, :, rows], vbuf.at[quad % NVSLOT, :, rows], vsem.at[slot])

    def start_kv(j):
        ksrc, kdst, ks, vsrc, vdst, vs = kv_refs(j // 2)
        base = (j % 2) * (STEP // 2)

        def one(c):
            rows = _ads(base + c * RROWS, RROWS, RROWS)
            copy(ksrc.at[:, rows], kdst.at[:, rows], ks).start(priority=0)
            copy(vsrc.at[:, rows], vdst.at[:, rows], vs).start(priority=1)

        _loop(STEP // 2 // RROWS, one, 8)

    def wait_kv(n):
        ksrc, kdst, ks, vsrc, vdst, vs = kv_refs(n)
        copy(ksrc, kdst, ks).wait()
        copy(vsrc, vdst, vs).wait()

    def start_unit(src, dst, rh, sem):
        def one(c):
            rows = _ads(rh * PART + c * WROWS, WROWS, WROWS)
            copy(src.at[:, rows], dst.at[:, rows], sem).start()

        _loop(PART // WROWS, one, 8)

    def wait_unit(src, dst, rh, sem):
        rows = _ads(rh * PART, PART, PART)
        copy(src.at[:, rows], dst.at[:, rows], sem).wait()

    def dv_unit(quad, rh):
        return vbuf.at[DVSLOT], dv_hbm.at[quad], rh, wsem.at[rh]

    def dk_unit(quad, rh):
        return vbuf.at[quad % NVSLOT], dk_hbm.at[quad], rh, wsem.at[2 + rh]

    in_pairs = ((x_hbm, x_s), (go_hbm, go_s), (b1_hbm, b1_s), (b2_hbm, b2_s),
                (wq_hbm, wq), (wo_hbm, wo), (w1_hbm, w1), (w2_hbm, w2))
    out_pairs = ((out_s, out_hbm), (db1_s, db1_hbm), (db2_s, db2_hbm), (dx_s, dx_hbm),
                 (dwq, dwq_hbm), (dwo, dwo_hbm), (dw1, dw1_hbm), (dw2, dw2_hbm))

    def in_copy(n):
        return copy(in_pairs[n][0], in_pairs[n][1], isem.at[n])

    def out_copy(n):
        return copy(out_pairs[n][0], out_pairs[n][1], osem.at[n])

    def start_attn_weights(r):
        qrows = _ads(r * 8, 8, 8)
        for c in range(8):
            qcols = pl.ds(c * 512, 512)
            orows = _ads(r * 64 + c * 8, 8, 8)
            copy(wq_hbm.at[:, qrows, qcols], wq.at[:, qrows, qcols], isem.at[4]).start(priority=0)
            copy(wo_hbm.at[:, orows], wo.at[:, orows], isem.at[5]).start(priority=1)

    def start_mlp_weights(r):
        for c in range(8):
            rows1 = _ads(r * 64 + c * 8, 8, 8)
            copy(w1_hbm.at[rows1], w1.at[rows1], isem.at[6]).start(priority=0)
            if c < 7:
                rows2 = _ads(r * 224 + c * 32, 32, 32)
                copy(w2_hbm.at[rows2], w2.at[rows2], isem.at[7]).start(priority=1)

    def start_weight_grads(r):
        for c in range(8):
            qrows = _ads(r * 16 + (c // 4) * 8, 8, 8)
            qcols = pl.ds((c % 4) * 1024, 1024)
            orows = _ads(r * 128 + c * 16, 16, 16)
            copy(dwq.at[:, qrows, qcols], dwq_hbm.at[:, qrows, qcols], osem.at[4]).start()
            copy(dwo.at[:, orows], dwo_hbm.at[:, orows], osem.at[5]).start()
            if c % 2 == 0:
                rows1 = _ads(r * 32 + (c // 2) * 8, 8, 8)
                copy(dw1.at[:, rows1], dw1_hbm.at[:, rows1], osem.at[6]).start()
            if c < 7:
                rows2 = _ads(r * 112 + c * 16, 16, 16)
                copy(dw2.at[:, rows2], dw2_hbm.at[:, rows2], osem.at[7]).start()

    for n in range(4):
        in_copy(n).start()
    _loop(16, start_attn_weights, 1)
    for ref in (o_all, dq_all, h_all, y_all, dh_all, g_all, da_all, acc_s, ksum_s, ml_s):
        ref[...] = jnp.zeros(ref.shape, F32)
    _loop(8, start_mlp_weights, 1)

    for n in range(6):
        in_copy(n).wait()
    xn2, _ = _ln(x_s[...].astype(F32))
    xn_all[...] = _pad_rows(xn2)
    xn_b16 = xn_all[...].astype(BF16)
    for c in range(HD // 1024):
        qc = slice(c * 1024, (c + 1) * 1024)
        q_all[:, qc] = _dot(xn_b16, wq[:, :, qc].reshape(D, 1024)).astype(BF16).astype(F32)
    start_kv(0)
    start_kv(1)
    in_copy(6).wait()
    in_copy(7).wait()
    dg_all[...] = _dot_nt(_pad_rows(go_s[...].astype(F32)).astype(BF16), w2[...])
    start_kv(2)

    def fwd_head(b, hs):
        site = b * (NSITE // B) + hs
        n = site // 2
        part = n % 4
        jq = hs // 8
        nxt = site + AHEAD

        @pl.when(site == NSITE // B + 2)
        def _():
            wait_unit(*dv_unit(QPB - 1, 0))
            wait_unit(*dv_unit(QPB - 1, 1))

        @pl.when(jnp.logical_and(nxt < NSITE, n != H))
        def _():
            start_kv(nxt)

        @pl.when(site == NSITE - 2)
        def _():
            start_unit(*dk_unit(QPB - 1, 0))
            start_unit(*dk_unit(QPB - 1, 1))

        @pl.when(site % 2 == 0)
        def _():
            wait_kv(n)

        first = part == 0
        for w in range(2):
            u = 2 * (site % 2) + w
            h = 4 * jq + u
            kref = kbuf.at[n % NKSLOT, pl.ds(2 * u, 2)]
            vref = vbuf.at[(n // 4) % NVSLOT, pl.ds(2 * u, 2), _ads(part * STEP, STEP, STEP)]
            q8 = jnp.broadcast_to(_get_row(q_all, b, _ads(h * DH, DH, DH)), (8, DH)).astype(BF16)
            s = _dot_nt(q8, kref[...].reshape(2 * STEP, DH)) * SCALE
            rows_all[part, pl.ds(h, 1), :] = s[0:1]
            m_old = jnp.where(first, -jnp.inf, ml_s[u, 0])
            m_new = jnp.maximum(m_old, jnp.max(s, axis=1, keepdims=True))
            alpha = jnp.exp(m_old - m_new)
            e = jnp.exp(s - m_new[:, 0:1])
            ml_s[u, 0] = m_new
            ml_s[u, 1] = jnp.where(first, 0.0, ml_s[u, 1] * alpha) + jnp.sum(e, axis=1, keepdims=True)
            e = e.astype(BF16).astype(F32)
            ml_s[u, 2] = jnp.where(first, 0.0, ml_s[u, 2] * alpha) + jnp.sum(e, axis=1, keepdims=True)
            acc = jnp.where(first, 0.0, acc_s[u] * alpha[0:1])
            ksum = jnp.where(first, 0.0, ksum_s[u] * alpha[0:1])
            for c in range(2 * STEP // CH):
                half, r = divmod(c * CH, STEP)
                ec = e[:, c * CH:(c + 1) * CH]
                a = (kref[half, r:r + CH, :].T.astype(F32) * ec[0:1]).astype(BF16)
                lhs = jnp.concatenate(
                    [a, jnp.concatenate([ec, ec], axis=0).astype(BF16)], axis=0)
                acc = acc + _dot(lhs, vref[half, r:r + CH, :])
                for j in range(CH // DH):
                    ksum = ksum + a[:, j * DH:(j + 1) * DH].astype(F32)
            acc_s[u] = acc
            ksum_s[u] = ksum

        @pl.when(part == 3)
        def _():
            for w in range(2):
                u = 2 * (site % 2) + w
                h = 4 * jq + u
                m = ml_s[u, 0][0:1]
                inv = 1.0 / ml_s[u, 1][0:1]
                for r in range(4):
                    rows_all[r, pl.ds(h, 1), :] = (
                        jnp.exp(rows_all[r, pl.ds(h, 1), :] - m[:, 0:1]) * inv[:, 0:1])
                inv = 1.0 / ml_s[u, 2][0:1]
                o8 = acc_s[u, DH:DH + 8, :] * inv
                kbar = jnp.sum(ksum_s[u], axis=1, keepdims=True) * inv
                m_all[h] = ((acc_s[u, 0:DH, :] * inv - kbar * o8[0:1]) * SCALE).astype(BF16)
                _set_row(o_all, b, _ads(h * DH, DH, DH), o8)
                att_s[...] += _dot(o8.astype(BF16), wo[h // 8, _ads((h % 8) * DH, DH, DH), :])

    def mlp_mid(b, att):
        row = pl.ds(b, 1)
        x2 = x_s[...].astype(F32)
        go2 = go_s[...].astype(F32)
        hh = att + jnp.where(b == 0, x2[0:1], x2[1:2])
        go = jnp.where(b == 0, go2[0:1], go2[1:2])
        hn, r1 = _ln(hh)
        y, r2 = _ln(hn)
        a = _dot(y.astype(BF16), w1[...]) + b1_s[...].astype(F32).reshape(1, FF)
        t = jnp.tanh(GELU_C * (a + GELU_A * a * a * a))
        dgelu = 0.5 * (1.0 + t) + 0.5 * a * (1.0 - t * t) * GELU_C * (1.0 + 3.0 * GELU_A * a * a)
        da = dg_all[row, :] * dgelu
        dy = _dot_nt(da.astype(BF16), w1[...])
        dh = go + _ln_bwd(_ln_bwd(dy, y, r2), hn, r1)
        h_all[row, :] = hh[0:1]
        y_all[row, :] = y[0:1]
        g_all[row, :] = (0.5 * a * (1.0 + t))[0:1]
        da_all[row, :] = da[0:1]
        dh_all[row, :] = dh[0:1]

    def mlp_outputs():
        go2 = go_s[...].astype(F32)
        g16 = g_all[...].astype(BF16)
        mlp = _dot(g16, w2[...]) + b2_s[...].astype(F32).reshape(1, D)
        out_s[...] = (h_all[...] + mlp)[0:B].astype(BF16)
        db1_s[...] = (da_all[0:1, :] + da_all[1:2, :]).reshape(FF).astype(BF16)
        db2_s[...] = (go2[0:1] + go2[1:2]).reshape(D).astype(BF16)
        for n in range(3):
            out_copy(n).start()
        go16 = _pad_rows(go2).astype(BF16)
        for c in range(FF // 128):
            dw2[c // 7, (c % 7) * 128:(c % 7 + 1) * 128, :] = _dot_tn(
                g16[:, c * 128:(c + 1) * 128], go16).astype(BF16)
        y16 = y_all[...].astype(BF16)
        da16 = da_all[...].astype(BF16)
        for c in range(D // 128):
            dw1[c // 2, (c % 2) * 128:(c % 2 + 1) * 128, :] = _dot_tn(
                y16[:, c * 128:(c + 1) * 128], da16).astype(BF16)

    def dwo_output():
        o16 = o_all[...].astype(BF16)
        dh16 = dh_all[...].astype(BF16)
        for c in range(HD // 256):
            dwo[c // 4, (c % 4) * 256:(c % 4 + 1) * 256, :] = _dot_tn(
                o16[:, c * 256:(c + 1) * 256], dh16).astype(BF16)

    def bwd_quad(b, jq):
        quad = b * QPB + jq
        slot = quad % NVSLOT
        qlanes = _ads(jq * 4 * DH, 4 * DH, 4 * DH)
        dh8 = jnp.broadcast_to(dh_all[pl.ds(b, 1), :], (8, D)).astype(BF16)
        do8 = _dot_nt(dh8, wo[jq // 2, _ads((jq % 2) * 4 * DH, 4 * DH, 4 * DH), :]).astype(BF16)
        q8 = jnp.broadcast_to(_get_row(q_all, b, qlanes) * SCALE, (8, 4 * DH))
        dq8 = []
        for u in range(4):
            ul = slice(u * DH, (u + 1) * DH)
            cols[0, u] = do8[:, ul].astype(F32)
            cols[1, u] = q8[:, ul]
            dq8.append(_dot_nt(do8[:, ul], m_all[4 * jq + u]))
        _set_row(dq_all, b, qlanes, jnp.concatenate(dq8, axis=1))

        def score_grad(u):
            dp = _dot_nt(cols[0, u].astype(BF16), vbuf[slot, pl.ds(2 * u, 2)].reshape(S, DH))[0:1]
            prow = pl.ds(4 * jq + u, 1)
            p = jnp.concatenate(
                [rows_all[r, prow, half * STEP:(half + 1) * STEP]
                 for half in range(2) for r in range(4)], axis=1)
            ds = p * (dp - jnp.sum(p * dp, axis=1, keepdims=True))
            for r in range(4):
                for half in range(2):
                    k0 = half * SROWS + r * STEP
                    rows_all[r, pl.ds(H + u, 1), half * STEP:(half + 1) * STEP] = ds[:, k0:k0 + STEP]

        def unit(t):
            kind = t // 2
            rh = t % 2

            @pl.when(t == 2)
            def _():
                _loop(4, score_grad, 1)

            @pl.when(jnp.logical_and(kind == 0, jq > 0))
            def _():
                wait_unit(*dv_unit(quad - 1, rh))

            @pl.when(jnp.logical_and(kind == 1, quad > 0))
            def _():
                wait_unit(*dk_unit(quad - 1, rh))

            dst = vbuf.at[jnp.where(kind == 0, DVSLOT, slot)]
            row0 = jnp.where(kind == 0, 4 * jq, H)
            for u in range(4):
                col = jnp.broadcast_to(cols[kind, u][0:1], (DH, DH)).T
                for half in range(2):
                    for c in range(PART // CH):
                        rr, l0 = divmod(c * CH, STEP)
                        l0 += half * STEP
                        dst[2 * u + half, _ads(rh * PART + c * CH, CH, CH), :] = _outer_tiles(
                            col, rows_all[2 * rh + rr, pl.ds(row0 + u, 1), l0:l0 + CH])

            @pl.when(kind == 0)
            def _():
                start_unit(*dv_unit(quad, rh))

            @pl.when(jnp.logical_and(kind == 1, quad != QPB - 1))
            def _():
                start_unit(*dk_unit(quad, rh))

        _loop(4, unit, 1)

        @pl.when(quad == QPB)
        def _():
            mlp_outputs()

        @pl.when(quad == QPB + 1)
        def _():
            dwo_output()

    def batch(b):
        att_s[...] = jnp.zeros((8, D), F32)
        _loop(NSITE // B, lambda hs: fwd_head(b, hs), 1)

        @pl.when(b == 0)
        def _():
            start_kv(NSITE // B + AHEAD)

        mlp_mid(b, att_s[...])

        @pl.when(b == 0)
        def _():
            start_kv(NSITE // B + AHEAD + 1)

        _loop(QPB, lambda jq: bwd_quad(b, jq), 1)

    _loop(B, batch, 1)

    dq16 = dq_all[...].astype(BF16)
    xn16 = xn_all[...].astype(BF16)
    for c in range(D // 128):
        for n in range(HD // 1024):
            qc = slice(n * 1024, (n + 1) * 1024)
            dwq[c, :, qc] = _dot_tn(xn16[:, c * 128:(c + 1) * 128], dq16[:, qc]).astype(BF16)
    dxn = _dot_nt(dq16, wq[...].reshape(D, HD))[0:B]
    xn, rstd = _ln(x_s[...].astype(F32))
    dx_s[...] = (dh_all[0:B, :] + _ln_bwd(dxn, xn, rstd)).astype(BF16)
    out_copy(3).start()
    _loop(8, start_weight_grads, 1)

    for rh in range(2):
        wait_unit(*dv_unit(NQUAD - 1, rh))
        wait_unit(*dk_unit(NQUAD - 1, rh))
    for n in range(len(out_pairs)):
        out_copy(n).wait()


@jax.jit
def pallas_sequential_preLN__mha_block_cached__mixer_channel_mlp__decode_kernel(
    A_x: jax.Array,
    A_k_cache: jax.Array,
    A_v_cache: jax.Array,
    A_wq: jax.Array,
    A_wo: jax.Array,
    B_x: jax.Array,
    B_w1: jax.Array,
    B_b1: jax.Array,
    B_w2: jax.Array,
    B_b2: jax.Array,
    grad_out: jax.Array,
):
    del B_x
    kv_shape = (NQUAD, 8, SROWS, DH)
    wq_shape = (4, D // 4, HD)
    wo_shape = (4, HD // 4, D)
    dw1_shape = (2, D // 2, FF)
    dw2_shape = (2, FF // 2, D)
    hbm = pl.BlockSpec(memory_space=pl.ANY)
    out_shape = tuple(
        jax.ShapeDtypeStruct(s, BF16)
        for s in ((B, D), (B, D), kv_shape, kv_shape, wq_shape, wo_shape,
                  dw1_shape, (FF,), dw2_shape, (D,)))
    vm = pltpu.VMEM
    dma = pltpu.SemaphoreType.DMA
    scratch = [
        vm((NKSLOT, 8, STEP, DH), BF16),
        vm((NVSLOT + 1, 8, SROWS, DH), BF16),
        vm(wq_shape, BF16), vm(wo_shape, BF16), vm((D, FF), BF16), vm((FF, D), BF16),
        vm(wq_shape, BF16), vm(wo_shape, BF16), vm(dw1_shape, BF16), vm(dw2_shape, BF16),
        vm((B, D), BF16), vm((B, D), BF16), vm((FF,), BF16), vm((D,), BF16),
        vm((B, D), BF16), vm((B, D), BF16), vm((FF,), BF16), vm((D,), BF16),
        vm((4, H + 8, 2 * STEP), F32), vm((H, DH, DH), BF16),
        vm((4, DH + RP, DH), F32), vm((4, DH, DH), F32), vm((4, 3, 8, DH), F32), vm((8, D), F32),
        vm((2, 4, 8, DH), F32),
        vm((RP, HD), F32), vm((RP, HD), F32), vm((RP, HD), F32),
        vm((RP, D), F32), vm((RP, D), F32), vm((RP, D), F32), vm((RP, D), F32),
        vm((RP, FF), F32), vm((RP, FF), F32), vm((RP, FF), F32),
        dma((NKSLOT,)), dma((NKSLOT,)), dma((4,)), dma((8,)), dma((8,)),
    ]
    out, dx, dk, dv, dwq, dwo, dw1, db1, dw2, db2 = pl.pallas_call(
        _kernel,
        out_shape=out_shape,
        in_specs=[hbm] * 10,
        out_specs=[hbm] * 10,
        scratch_shapes=scratch,
        compiler_params=pltpu.CompilerParams(vmem_limit_bytes=124 * 2**20, disable_bounds_checks=True),
    )(A_x.reshape(B, D), A_k_cache.reshape(kv_shape), A_v_cache.reshape(kv_shape),
      A_wq.reshape(wq_shape), A_wo.reshape(wo_shape), B_w1, B_b1, B_w2, B_b2,
      grad_out.reshape(B, D))
    return (out.reshape(A_x.shape), dx.reshape(A_x.shape), dk.reshape(A_k_cache.shape),
            dv.reshape(A_v_cache.shape), dwq.reshape(A_wq.shape), dwo.reshape(A_wo.shape),
            dw1.reshape(B_w1.shape), db1, dw2.reshape(B_w2.shape), db2)
```

```python
import jax
import jax.numpy as jnp
from jax import lax
import jax.experimental.pallas as pl
import jax.experimental.pallas.tpu as pltpu

F32 = jnp.float32
BF16 = jnp.bfloat16

B, H, S, DH = 2, 32, 8192, 128
D, FF = 512, 1792
HD = H * DH
NSTEP = B * H
NSITE = 2 * NSTEP
NQUAD = B * H // 4
QPB = H // 4
SROWS = S // 2
PART = SROWS // 2
STEP = SROWS // 4
AHEAD = 3
NVSLOT = QPB + 1
DVSLOT = NVSLOT
NKSLOT = 3
RROWS = 16
WROWS = 64
NP = STEP // (4 * RROWS)
LEAD = 13
RTAIL = 14
ROT = 3
WRAPQ = 3
CH = 256
RP = 16
SCALE = DH ** -0.5
EPS = 1e-5
GELU_C = 0.7978845608028654
GELU_A = 0.044715

NT = (((1,), (1,)), ((), ()))
TN = (((0,), (0,)), ((), ()))


def _dot(a, b):
    return jnp.dot(a, b, preferred_element_type=F32)


def _dot_nt(a, b):
    return lax.dot_general(a, b, NT, preferred_element_type=F32)


def _dot_tn(a, b):
    return lax.dot_general(a, b, TN, preferred_element_type=F32)


def _ln(x):
    mu = jnp.mean(x, axis=-1, keepdims=True)
    xc = x - mu
    var = jnp.mean(xc * xc, axis=-1, keepdims=True)
    rstd = lax.rsqrt(var + EPS)
    return xc * rstd, rstd


def _ln_bwd(dy, y, rstd):
    m1 = jnp.mean(dy, axis=-1, keepdims=True)
    m2 = jnp.mean(dy * y, axis=-1, keepdims=True)
    return (dy - m1 - y * m2) * rstd


def _pad_rows(x2):
    r = lax.broadcasted_iota(jnp.int32, (RP, x2.shape[1]), 0)
    return jnp.where(r == 0, x2[0:1], jnp.where(r == 1, x2[1:2], 0.0))


def _get_row(ref, b, lanes):
    blk = ref[0:8, lanes]
    return jnp.where(b == 0, blk[0:1], blk[1:2])


def _set_row(ref, b, lanes, val8):
    r = lax.broadcasted_iota(jnp.int32, val8.shape, 0)
    ref[0:8, lanes] = jnp.where(r == b, val8, ref[0:8, lanes])


def _outer_tiles(col, row):
    tiles = [col * row[:, j * DH:(j + 1) * DH] for j in range(row.shape[1] // DH)]
    return jnp.concatenate(tiles, axis=1).astype(BF16).T


def _ads(start, size, align):
    return pl.ds(pl.multiple_of(start, align), size)


def _loop(n, body, unroll=1):
    def wrapped(i, c):
        body(i)
        return c

    lax.fori_loop(0, n, wrapped, 0, unroll=unroll)


def _head_of(jq, u):
    return (4 * (jq + QPB - 1 - WRAPQ) + ROT + u) % H


def _head_lanes(jq, u):
    return _ads(_head_of(jq, u) * DH, DH, DH)


def _by_wrap(quads, fn):
    if not quads:
        fn()
        return

    def rest(w):
        _by_wrap(quads[1:], lambda *ws: fn(w, *ws))

    is_wrap = quads[0] % QPB == WRAPQ
    if isinstance(is_wrap, bool):
        rest(is_wrap)
    else:
        pl.when(is_wrap)(lambda: rest(True))
        pl.when(jnp.logical_not(is_wrap))(lambda: rest(False))


def _kernel(x_hbm, k_hbm, v_hbm, wq_hbm, wo_hbm, w1_hbm, b1_hbm, w2_hbm, b2_hbm, go_hbm,
            out_hbm, dx_hbm, dk_hbm, dv_hbm, dwq_hbm, dwo_hbm, dw1_hbm, db1_hbm, dw2_hbm, db2_hbm,
            kbuf, vbuf, wq, wo, w1, w2, dwq, dwo, dw1, dw2,
            x_s, go_s, b1_s, b2_s, out_s, dx_s, db1_s, db2_s,
            rows_all, m_all, acc_s, ksum_s, ml_s, att_s, cols,
            q_all, o_all, dq_all, xn_all, h_all, y_all, dh_all, g_all, da_all, dg_all,
            ksem, vsem, wsem, isem, osem):
    copy = pltpu.make_async_copy

    def wo_rows(jq, u):
        h = _head_of(jq, u)
        return wo[h // 8, _ads((h % 8) * DH, DH, DH), :]


    def k_dst(n):
        return kbuf.at[n % NKSLOT], ksem.at[n % NKSLOT]

    def v_dst(n):
        rows = _ads((n % 4) * STEP, STEP, STEP)
        return vbuf.at[(n // 4) % NVSLOT, :, rows], vsem.at[n % NKSLOT]

    def reader(hbm_ref, dst_fn, j, wrap):
        n = j // 2
        jq = (n // 4) % QPB
        s0 = (n // H) * 2 * H
        dst, sem = dst_fn(n)
        lo = (j % 2) * (STEP // 2)
        hi = (n % 4) * STEP + lo

        def piece(c, v):
            if wrap:
                u, ns, r, size = 2 * (c % 2) + v, 2, 4 * RROWS * (c // 2), 4 * RROWS
            else:
                u, ns, r, size = 0, 8, RROWS * (2 * c + v), RROWS
            return copy(hbm_ref.at[pl.ds(s0 + 2 * _head_of(jq, u), ns), _ads(hi + r, size, RROWS)],
                        dst.at[pl.ds(2 * u, ns), _ads(lo + r, size, RROWS)], sem)

        return piece

    def start_kv(j, last=False, inline=False):
        def run(n, body):
            if inline:
                for c in range(n):
                    body(c)
            else:
                _loop(n, body)

        def same(w):
            kp, vp = reader(k_hbm, k_dst, j, w), reader(v_hbm, v_dst, j, w)

            def one(c):
                for v in range(2):
                    kp(c, v).start(priority=0)
                    vp(c + LEAD, v).start(priority=1)

            run(NP - LEAD, one)

        def lead(wk, wv=None):
            kp = reader(k_hbm, k_dst, j, wk)
            vp = None if last else reader(v_hbm, v_dst, j + 1, wv)

            def one(c):
                for v in range(2):
                    kp(c + NP - LEAD, v).start(priority=0)
                    if not last:
                        vp(c, v).start(priority=1)

            run(LEAD, one)

        _by_wrap([j // 8], same)
        _by_wrap([j // 8] if last else [j // 8, (j + 1) // 8], lead)

    def start_v_head():
        vp = reader(v_hbm, v_dst, 0, False)

        def one(c):
            for v in range(2):
                vp(c, v).start(priority=v)

        _loop(LEAD, one)

    def wait_all(buf, sem):
        copy(buf, buf, sem).wait()

    def wait_v_pairs(n, c0, c1):
        vp = reader(v_hbm, v_dst, 2 * n, False)

        def one(c):
            for v in range(2):
                vp(c0 + c, v).wait()

        _loop(c1 - c0, one)


    def unit_parts(src, hbm_ref, quad, t, wrap):
        s0 = (quad // QPB) * 2 * H
        if not wrap:
            return [(src, hbm_ref.at[pl.ds(s0 + 2 * _head_of(quad % QPB, 0), 8)], wsem.at[t])]
        na = 8 - 2 * ROT
        return [(src.at[pl.ds(0, na)], hbm_ref.at[pl.ds(s0 + 2 * H - na, na)], wsem.at[t]),
                (src.at[pl.ds(na, 8 - na)], hbm_ref.at[pl.ds(s0, 8 - na)], wsem.at[4 + t])]

    def start_unit(src, hbm_ref, quad, rh, t):
        def go(w):
            parts = unit_parts(src, hbm_ref, quad, t, w)

            def one(c):
                rows = _ads(rh * PART + c * WROWS, WROWS, WROWS)
                for s, d, sem in parts:
                    copy(s.at[:, rows], d.at[:, rows], sem).start()

            _loop(PART // WROWS, one, 2)

        _by_wrap([quad], go)

    def wait_unit(src, hbm_ref, quad, rh, t):
        def go(w):
            rows = _ads(rh * PART, PART, PART)
            for s, d, sem in unit_parts(src, hbm_ref, quad, t, w):
                copy(s.at[:, rows], d.at[:, rows], sem).wait()

        _by_wrap([quad], go)

    def dv_unit(quad, rh):
        return vbuf.at[DVSLOT], dv_hbm, quad, rh, rh

    def dk_unit(quad, rh):
        return vbuf.at[quad % NVSLOT], dk_hbm, quad, rh, 2 + rh


    in_pairs = ((x_hbm, x_s), (go_hbm, go_s), (b1_hbm, b1_s), (b2_hbm, b2_s),
                (wq_hbm, wq), (wo_hbm, wo), (w1_hbm, w1), (w2_hbm, w2))
    out_pairs = ((out_s, out_hbm), (db1_s, db1_hbm), (db2_s, db2_hbm), (dx_s, dx_hbm),
                 (dwq, dwq_hbm), (dwo, dwo_hbm), (dw1, dw1_hbm), (dw2, dw2_hbm))

    def in_copy(n):
        return copy(in_pairs[n][0], in_pairs[n][1], isem.at[n])

    def out_copy(n):
        return copy(out_pairs[n][0], out_pairs[n][1], osem.at[n])

    def start_attn_weights(r):
        qrows = _ads(r * 8, 8, 8)
        for c in range(8):
            qcols = pl.ds(c * 512, 512)
            orows = _ads(r * 64 + c * 8, 8, 8)
            copy(wq_hbm.at[:, qrows, qcols], wq.at[:, qrows, qcols], isem.at[4]).start(priority=0)
            copy(wo_hbm.at[:, orows], wo.at[:, orows], isem.at[5]).start(priority=1)

    def start_mlp_weights(r):
        for c in range(8):
            rows1 = _ads(r * 64 + c * 8, 8, 8)
            copy(w1_hbm.at[rows1], w1.at[rows1], isem.at[6]).start(priority=0)
            if c < 7:
                rows2 = _ads(r * 224 + c * 32, 32, 32)
                copy(w2_hbm.at[rows2], w2.at[rows2], isem.at[7]).start(priority=1)

    def start_attn_grads(r):
        for c in range(8):
            qrows = _ads(r * 16 + (c // 4) * 8, 8, 8)
            qcols = pl.ds((c % 4) * 1024, 1024)
            orows = _ads(r * 128 + c * 16, 16, 16)
            copy(dwq.at[:, qrows, qcols], dwq_hbm.at[:, qrows, qcols], osem.at[4]).start()
            copy(dwo.at[:, orows], dwo_hbm.at[:, orows], osem.at[5]).start()

    def start_mlp_grads(r):
        for c in range(7):
            if c % 2 == 0:
                rows1 = _ads(r * 32 + (c // 2) * 8, 8, 8)
                copy(dw1.at[:, rows1], dw1_hbm.at[:, rows1], osem.at[6]).start()
            rows2 = _ads(r * 112 + c * 16, 16, 16)
            copy(dw2.at[:, rows2], dw2_hbm.at[:, rows2], osem.at[7]).start()


    for n in range(4):
        in_copy(n).start()
    _loop(16, start_attn_weights)
    for ref in (o_all, dq_all, h_all, y_all, dh_all, g_all, da_all, acc_s, ksum_s, ml_s):
        ref[...] = jnp.zeros(ref.shape, F32)
    _loop(8, start_mlp_weights)
    for n in range(6):
        in_copy(n).wait()
    xn_all[...] = _pad_rows(_ln(x_s[...].astype(F32))[0])
    xn_b16 = xn_all[...].astype(BF16)
    for c in range(HD // 1024):
        qc = slice(c * 1024, (c + 1) * 1024)
        q_all[:, qc] = _dot(xn_b16, wq[:, :, qc].reshape(D, 1024)).astype(BF16).astype(F32)
    start_v_head()
    start_kv(0)
    start_kv(1)
    in_copy(6).wait()
    in_copy(7).wait()
    dg_all[...] = _dot_nt(_pad_rows(go_s[...].astype(F32)).astype(BF16), w2[...])
    start_kv(2)

    split_step = (NSITE // B + AHEAD + 2) // 2
    split_pairs = NP + LEAD - RTAIL // 2


    def fwd_half(b, hs):
        site = b * (NSITE // B) + hs
        n = site // 2
        part = n % 4
        jq = hs // 8
        nxt = site + AHEAD

        @pl.when(site == NSITE // B + 2)
        def _():
            wait_unit(*dv_unit(QPB - 1, 0))
            wait_unit(*dv_unit(QPB - 1, 1))

        @pl.when(jnp.logical_and(nxt < NSITE - 1, n != H))
        def _():
            start_kv(nxt, inline=True)

        @pl.when(nxt == NSITE - 1)
        def _():
            start_kv(NSITE - 1, last=True)

        @pl.when(site == NSITE - 3)
        def _():
            wait_v_pairs(NSTEP - 1, 0, 2 * NP - RTAIL // 2)
            start_unit(*dk_unit(QPB - 1, 0))
            start_unit(*dk_unit(QPB - 1, 1))

        @pl.when(site % 2 == 0)
        def _():
            wait_all(*k_dst(n))

            @pl.when(jnp.logical_and(n != split_step, n != NSTEP - 1))
            def _():
                wait_all(*v_dst(n))

            @pl.when(n == split_step)
            def _():
                wait_v_pairs(split_step, split_pairs, 2 * NP)

            @pl.when(n == NSTEP - 1)
            def _():
                wait_v_pairs(NSTEP - 1, 2 * NP - RTAIL // 2, 2 * NP)

        first = part == 0
        heads = []
        for w in range(2):
            u = 2 * (site % 2) + w
            kref = kbuf.at[n % NKSLOT, pl.ds(2 * u, 2)]
            q8 = jnp.broadcast_to(_get_row(q_all, b, _head_lanes(jq, u)), (8, DH)).astype(BF16)
            s = _dot_nt(q8, kref[...].reshape(2 * STEP, DH)) * SCALE
            rows_all[part, pl.ds(4 * jq + u, 1), :] = s[0:1]
            m_old = jnp.where(first, -jnp.inf, ml_s[u, 0])
            m_new = jnp.maximum(m_old, jnp.max(s, axis=1, keepdims=True))
            alpha = jnp.exp(m_old - m_new)
            e = jnp.exp(s - m_new[:, 0:1])
            ml_s[u, 0] = m_new
            ml_s[u, 1] = jnp.where(first, 0.0, ml_s[u, 1] * alpha) + jnp.sum(e, axis=1, keepdims=True)
            e = e.astype(BF16).astype(F32)
            ml_s[u, 2] = jnp.where(first, 0.0, ml_s[u, 2] * alpha) + jnp.sum(e, axis=1, keepdims=True)
            heads.append((u, kref, e, alpha[0:1]))

        for u, kref, e, alpha in heads:
            vref = vbuf.at[(n // 4) % NVSLOT, pl.ds(2 * u, 2), _ads(part * STEP, STEP, STEP)]
            acc = jnp.where(first, 0.0, acc_s[u] * alpha)
            ksum = jnp.where(first, 0.0, ksum_s[u] * alpha)
            for half in range(2):
                ec = e[:, half * STEP:(half + 1) * STEP]
                lhs = jnp.concatenate(
                    [kref[half].T.astype(F32) * ec[0:1], ec, ec], axis=0).astype(BF16)
                acc = acc + _dot(lhs, vref[half])
                for j in range(STEP // DH):
                    ksum = ksum + lhs[0:DH, j * DH:(j + 1) * DH].astype(F32)
            acc_s[u] = acc
            ksum_s[u] = ksum

        @pl.when(part == 3)
        def _():
            for w in range(2):
                u = 2 * (site % 2) + w
                prow = pl.ds(4 * jq + u, 1)
                m = ml_s[u, 0][0:1, 0:1]
                inv_p = 1.0 / ml_s[u, 1][0:1, 0:1]
                for r in range(4):
                    rows_all[r, prow, :] = jnp.exp(rows_all[r, prow, :] - m) * inv_p
                inv = 1.0 / ml_s[u, 2][0:1]
                o8 = acc_s[u, DH:DH + 8, :] * inv
                kbar = jnp.sum(ksum_s[u], axis=1, keepdims=True) * inv
                m_all[4 * jq + u] = ((acc_s[u, 0:DH, :] * inv - kbar * o8[0:1]) * SCALE).astype(BF16)
                _set_row(o_all, b, _head_lanes(jq, u), o8)
                att_s[...] += _dot(o8.astype(BF16), wo_rows(jq, u))


    def mlp_mid(b):
        row = pl.ds(b, 1)
        x2 = x_s[...].astype(F32)
        go2 = go_s[...].astype(F32)
        hh = att_s[...] + jnp.where(b == 0, x2[0:1], x2[1:2])
        go = jnp.where(b == 0, go2[0:1], go2[1:2])
        hn, r1 = _ln(hh)
        y, r2 = _ln(hn)
        a = _dot(y.astype(BF16), w1[...]) + b1_s[...].astype(F32).reshape(1, FF)
        t = jnp.tanh(GELU_C * (a + GELU_A * a * a * a))
        dgelu = 0.5 * (1.0 + t) + 0.5 * a * (1.0 - t * t) * GELU_C * (1.0 + 3.0 * GELU_A * a * a)
        da = dg_all[row, :] * dgelu
        dy = _dot_nt(da.astype(BF16), w1[...])
        dh = go + _ln_bwd(_ln_bwd(dy, y, r2), hn, r1)
        h_all[row, :] = hh[0:1]
        y_all[row, :] = y[0:1]
        g_all[row, :] = (0.5 * a * (1.0 + t))[0:1]
        da_all[row, :] = da[0:1]
        dh_all[row, :] = dh[0:1]

    def mlp_outputs():
        go2 = go_s[...].astype(F32)
        g16 = g_all[...].astype(BF16)
        mlp = _dot(g16, w2[...]) + b2_s[...].astype(F32).reshape(1, D)
        out_s[...] = (h_all[...] + mlp)[0:B].astype(BF16)
        db1_s[...] = (da_all[0:1, :] + da_all[1:2, :]).reshape(FF).astype(BF16)
        db2_s[...] = (go2[0:1] + go2[1:2]).reshape(D).astype(BF16)
        for n in range(3):
            out_copy(n).start()
        go16 = _pad_rows(go2).astype(BF16)
        for c in range(FF // 128):
            dw2[c // 7, (c % 7) * 128:(c % 7 + 1) * 128, :] = _dot_tn(
                g16[:, c * 128:(c + 1) * 128], go16).astype(BF16)
        y16 = y_all[...].astype(BF16)
        da16 = da_all[...].astype(BF16)
        for c in range(D // 128):
            dw1[c // 2, (c % 2) * 128:(c % 2 + 1) * 128, :] = _dot_tn(
                y16[:, c * 128:(c + 1) * 128], da16).astype(BF16)

    def dwo_output():
        o16 = o_all[...].astype(BF16)
        dh16 = dh_all[...].astype(BF16)
        for c in range(HD // 256):
            dwo[c // 4, (c % 4) * 256:(c % 4 + 1) * 256, :] = _dot_tn(
                o16[:, c * 256:(c + 1) * 256], dh16).astype(BF16)


    def bwd_quad(b, jq):
        quad = b * QPB + jq
        slot = quad % NVSLOT
        dh8 = jnp.broadcast_to(dh_all[pl.ds(b, 1), :], (8, D)).astype(BF16)
        for u in range(4):
            cols[0, u] = _dot_nt(dh8, wo_rows(jq, u)).astype(BF16).astype(F32)
            cols[1, u] = jnp.broadcast_to(_get_row(q_all, b, _head_lanes(jq, u)) * SCALE, (8, DH))

        def score_grad(u):
            do8 = cols[0, u].astype(BF16)
            _set_row(dq_all, b, _head_lanes(jq, u), _dot_nt(do8, m_all[4 * jq + u]))
            dp = _dot_nt(do8, vbuf[slot, pl.ds(2 * u, 2)].reshape(S, DH))[0:1]
            prow = pl.ds(4 * jq + u, 1)
            p = jnp.concatenate(
                [rows_all[r, prow, half * STEP:(half + 1) * STEP]
                 for half in range(2) for r in range(4)], axis=1)
            ds = p * (dp - jnp.sum(p * dp, axis=1, keepdims=True))
            for r in range(4):
                for half in range(2):
                    k0 = half * SROWS + r * STEP
                    rows_all[r, pl.ds(H + u, 1), half * STEP:(half + 1) * STEP] = ds[:, k0:k0 + STEP]

        def unit(t):
            kind = t // 2
            rh = t % 2

            @pl.when(jnp.logical_or(t == 1, t == 2))
            def _():
                _loop(2, lambda w: score_grad(2 * (t - 1) + w))

            @pl.when(jnp.logical_and(kind == 0, jq > 0))
            def _():
                wait_unit(*dv_unit(quad - 1, rh))

            @pl.when(jnp.logical_and(kind == 1, quad > 0))
            def _():
                wait_unit(*dk_unit(quad - 1, rh))

            dst = vbuf.at[jnp.where(kind == 0, DVSLOT, slot)]
            row0 = jnp.where(kind == 0, 4 * jq, H)
            for u in range(4):
                col = jnp.broadcast_to(cols[kind, u][0:1], (DH, DH)).T
                for half in range(2):
                    for c in range(PART // CH):
                        rr, l0 = divmod(c * CH, STEP)
                        l0 += half * STEP
                        dst[2 * u + half, _ads(rh * PART + c * CH, CH, CH), :] = _outer_tiles(
                            col, rows_all[2 * rh + rr, pl.ds(row0 + u, 1), l0:l0 + CH])

            @pl.when(jnp.logical_and(quad == 0, t == 0))
            def _():
                wait_v_pairs(split_step, 0, split_pairs)

            @pl.when(kind == 0)
            def _():
                start_unit(*dv_unit(quad, rh))

            @pl.when(jnp.logical_and(kind == 1, quad != QPB - 1))
            def _():
                start_unit(*dk_unit(quad, rh))

        _loop(4, unit)

        @pl.when(quad == QPB)
        def _():
            mlp_outputs()

        @pl.when(quad == QPB + 1)
        def _():
            dwo_output()

    def batch(b):
        att_s[...] = jnp.zeros((8, D), F32)
        _loop(NSITE // B, lambda hs: fwd_half(b, hs))

        @pl.when(b == 0)
        def _():
            start_kv(NSITE // B + AHEAD)

        mlp_mid(b)

        @pl.when(b == 0)
        def _():
            start_kv(NSITE // B + AHEAD + 1)

        _loop(QPB, lambda jq: bwd_quad(b, jq))

    _loop(B, batch)


    dq16 = dq_all[...].astype(BF16)
    xn16 = xn_all[...].astype(BF16)
    for c in range(D // 128):
        for n in range(HD // 1024):
            qc = slice(n * 1024, (n + 1) * 1024)
            dwq[c, :, qc] = _dot_tn(xn16[:, c * 128:(c + 1) * 128], dq16[:, qc]).astype(BF16)
    dxn = _dot_nt(dq16, wq[...].reshape(D, HD))[0:B]
    xn, rstd = _ln(x_s[...].astype(F32))
    dx_s[...] = (dh_all[0:B, :] + _ln_bwd(dxn, xn, rstd)).astype(BF16)
    out_copy(3).start()
    _loop(8, start_attn_grads)
    _loop(8, start_mlp_grads)

    for rh in range(2):
        wait_unit(*dv_unit(NQUAD - 1, rh))
        wait_unit(*dk_unit(NQUAD - 1, rh))
    for n in range(len(out_pairs)):
        out_copy(n).wait()


@jax.jit
def pallas_sequential_preLN__mha_block_cached__mixer_channel_mlp__decode_kernel(
    A_x: jax.Array,
    A_k_cache: jax.Array,
    A_v_cache: jax.Array,
    A_wq: jax.Array,
    A_wo: jax.Array,
    B_x: jax.Array,
    B_w1: jax.Array,
    B_b1: jax.Array,
    B_w2: jax.Array,
    B_b2: jax.Array,
    grad_out: jax.Array,
):
    del B_x
    kv_shape = (2 * B * H, SROWS, DH)
    wq_shape = (4, D // 4, HD)
    wo_shape = (4, HD // 4, D)
    dw1_shape = (2, D // 2, FF)
    dw2_shape = (2, FF // 2, D)
    hbm = pl.BlockSpec(memory_space=pl.ANY)
    out_shape = tuple(
        jax.ShapeDtypeStruct(s, BF16)
        for s in ((B, D), (B, D), kv_shape, kv_shape, wq_shape, wo_shape,
                  dw1_shape, (FF,), dw2_shape, (D,)))
    vm = pltpu.VMEM
    dma = pltpu.SemaphoreType.DMA
    scratch = [
        vm((NKSLOT, 8, STEP, DH), BF16),
        vm((NVSLOT + 1, 8, SROWS, DH), BF16),
        vm(wq_shape, BF16), vm(wo_shape, BF16), vm((D, FF), BF16), vm((FF, D), BF16),
        vm(wq_shape, BF16), vm(wo_shape, BF16), vm(dw1_shape, BF16), vm(dw2_shape, BF16),
        vm((B, D), BF16), vm((B, D), BF16), vm((FF,), BF16), vm((D,), BF16),
        vm((B, D), BF16), vm((B, D), BF16), vm((FF,), BF16), vm((D,), BF16),
        vm((4, H + 8, 2 * STEP), F32), vm((H, DH, DH), BF16),
        vm((4, DH + RP, DH), F32), vm((4, DH, DH), F32), vm((4, 3, 8, DH), F32),
        vm((8, D), F32), vm((2, 4, 8, DH), F32),
        vm((RP, HD), F32), vm((RP, HD), F32), vm((RP, HD), F32),
        vm((RP, D), F32), vm((RP, D), F32), vm((RP, D), F32), vm((RP, D), F32),
        vm((RP, FF), F32), vm((RP, FF), F32), vm((RP, FF), F32),
        dma((NKSLOT,)), dma((NKSLOT,)), dma((8,)), dma((8,)), dma((8,)),
    ]
    out, dx, dk, dv, dwq, dwo, dw1, db1, dw2, db2 = pl.pallas_call(
        _kernel,
        out_shape=out_shape,
        in_specs=[hbm] * 10,
        out_specs=[hbm] * 10,
        scratch_shapes=scratch,
        compiler_params=pltpu.CompilerParams(
            vmem_limit_bytes=124 * 2**20, disable_bounds_checks=True),
    )(A_x.reshape(B, D), A_k_cache.reshape(kv_shape), A_v_cache.reshape(kv_shape),
      A_wq.reshape(wq_shape), A_wo.reshape(wo_shape), B_w1, B_b1, B_w2, B_b2,
      grad_out.reshape(B, D))
    return (out.reshape(A_x.shape), dx.reshape(A_x.shape), dk.reshape(A_k_cache.shape),
            dv.reshape(A_v_cache.shape), dwq.reshape(A_wq.shape), dwo.reshape(A_wo.shape),
            dw1.reshape(B_w1.shape), db1, dw2.reshape(B_w2.shape), db2)
```

```python
import jax
import jax.numpy as jnp
from jax import lax
import jax.experimental.pallas as pl
import jax.experimental.pallas.tpu as pltpu

F32 = jnp.float32
BF16 = jnp.bfloat16

B, H, S, DH = 2, 32, 8192, 128
D, FF = 512, 1792
HD = H * DH
NSTEP = B * H
NSITE = 2 * NSTEP
NQUAD = B * H // 4
QPB = H // 4
SROWS = S // 2
PART = SROWS // 2
STEP = SROWS // 4
AHEAD = 3
NVSLOT = QPB + 1
DVSLOT = NVSLOT
NKSLOT = 3
RROWS = 16
WROWS = 64
NP = STEP // (4 * RROWS)
LEAD = 13
RTAIL = 14
ROT = 3
WRAPQ = 3
CH = 256
RP = 16
SCALE = DH ** -0.5
EPS = 1e-5
GELU_C = 0.7978845608028654
GELU_A = 0.044715

NT = (((1,), (1,)), ((), ()))
TN = (((0,), (0,)), ((), ()))


def _dot(a, b):
    return jnp.dot(a, b, preferred_element_type=F32)


def _dot_nt(a, b):
    return lax.dot_general(a, b, NT, preferred_element_type=F32)


def _dot_tn(a, b):
    return lax.dot_general(a, b, TN, preferred_element_type=F32)


def _ln(x):
    mu = jnp.mean(x, axis=-1, keepdims=True)
    xc = x - mu
    var = jnp.mean(xc * xc, axis=-1, keepdims=True)
    rstd = lax.rsqrt(var + EPS)
    return xc * rstd, rstd


def _ln_bwd(dy, y, rstd):
    m1 = jnp.mean(dy, axis=-1, keepdims=True)
    m2 = jnp.mean(dy * y, axis=-1, keepdims=True)
    return (dy - m1 - y * m2) * rstd


def _pad_rows(x2):
    r = lax.broadcasted_iota(jnp.int32, (RP, x2.shape[1]), 0)
    return jnp.where(r == 0, x2[0:1], jnp.where(r == 1, x2[1:2], 0.0))


def _get_row(ref, b, lanes):
    blk = ref[0:8, lanes]
    return jnp.where(b == 0, blk[0:1], blk[1:2])


def _set_row(ref, b, lanes, val8):
    r = lax.broadcasted_iota(jnp.int32, val8.shape, 0)
    ref[0:8, lanes] = jnp.where(r == b, val8, ref[0:8, lanes])


def _outer_tiles(col, row):
    tiles = [col * row[:, j * DH:(j + 1) * DH] for j in range(row.shape[1] // DH)]
    return jnp.concatenate(tiles, axis=1).astype(BF16).T


def _ads(start, size, align):
    return pl.ds(pl.multiple_of(start, align), size)


def _loop(n, body, unroll=1):
    def wrapped(i, c):
        body(i)
        return c

    lax.fori_loop(0, n, wrapped, 0, unroll=unroll)


def _head_of(jq, u):
    return (4 * (jq + QPB - 1 - WRAPQ) + ROT + u) % H


def _head_lanes(jq, u):
    return _ads(_head_of(jq, u) * DH, DH, DH)


def _by_wrap(quads, fn):
    if not quads:
        fn()
        return

    def rest(w):
        _by_wrap(quads[1:], lambda *ws: fn(w, *ws))

    is_wrap = quads[0] % QPB == WRAPQ
    if isinstance(is_wrap, bool):
        rest(is_wrap)
    else:
        pl.when(is_wrap)(lambda: rest(True))
        pl.when(jnp.logical_not(is_wrap))(lambda: rest(False))


def _kernel(x_hbm, k_hbm, v_hbm, wq_hbm, wo_hbm, w1_hbm, b1_hbm, w2_hbm, b2_hbm, go_hbm,
            out_hbm, dx_hbm, dk_hbm, dv_hbm, dwq_hbm, dwo_hbm, dw1_hbm, db1_hbm, dw2_hbm, db2_hbm,
            kbuf, vbuf, wq, wo, w1, w2, dwq, dwo, dw1, dw2,
            x_s, go_s, b1_s, b2_s, out_s, dx_s, db1_s, db2_s,
            rows_all, m_all, acc_s, ksum_s, ml_s, att_s, cols,
            q_all, o_all, dq_all, xn_all, h_all, y_all, dh_all, g_all, da_all, dg_all,
            ksem, vsem, wsem, isem, osem):
    copy = pltpu.make_async_copy

    def wo_rows(jq, u):
        h = _head_of(jq, u)
        return wo[h // 8, _ads((h % 8) * DH, DH, DH), :]


    def k_dst(n):
        return kbuf.at[n % NKSLOT], ksem.at[n % NKSLOT]

    def v_dst(n):
        rows = _ads((n % 4) * STEP, STEP, STEP)
        return vbuf.at[(n // 4) % NVSLOT, :, rows], vsem.at[n % NKSLOT]

    def reader(hbm_ref, dst_fn, j, wrap):
        n = j // 2
        jq = (n // 4) % QPB
        s0 = (n // H) * 2 * H
        dst, sem = dst_fn(n)
        lo = (j % 2) * (STEP // 2)
        hi = (n % 4) * STEP + lo

        def piece(c, v):
            if wrap:
                u, ns, r, size = 2 * (c % 2) + v, 2, 4 * RROWS * (c // 2), 4 * RROWS
            else:
                u, ns, r, size = 0, 8, RROWS * (2 * c + v), RROWS
            return copy(hbm_ref.at[pl.ds(s0 + 2 * _head_of(jq, u), ns), _ads(hi + r, size, RROWS)],
                        dst.at[pl.ds(2 * u, ns), _ads(lo + r, size, RROWS)], sem)

        return piece

    def start_kv(j, last=False, inline=False):
        def run(n, body):
            if inline:
                for c in range(n):
                    body(c)
            else:
                _loop(n, body)

        def same(w):
            kp, vp = reader(k_hbm, k_dst, j, w), reader(v_hbm, v_dst, j, w)

            def one(c):
                for v in range(2):
                    kp(c, v).start(priority=0)
                    vp(c + LEAD, v).start(priority=1)

            run(NP - LEAD, one)

        def lead(wk, wv=None):
            kp = reader(k_hbm, k_dst, j, wk)
            vp = None if last else reader(v_hbm, v_dst, j + 1, wv)

            def one(c):
                for v in range(2):
                    kp(c + NP - LEAD, v).start(priority=0)
                    if not last:
                        vp(c, v).start(priority=1)

            run(LEAD, one)

        _by_wrap([j // 8], same)
        _by_wrap([j // 8] if last else [j // 8, (j + 1) // 8], lead)

    def start_v_head():
        vp = reader(v_hbm, v_dst, 0, False)

        def one(c):
            for v in range(2):
                vp(c, v).start(priority=v)

        _loop(LEAD, one)

    def wait_all(buf, sem):
        copy(buf, buf, sem).wait()

    def wait_v_pairs(n, c0, c1):
        vp = reader(v_hbm, v_dst, 2 * n, False)

        def one(c):
            for v in range(2):
                vp(c0 + c, v).wait()

        _loop(c1 - c0, one)


    def unit_parts(src, hbm_ref, quad, t, wrap):
        s0 = (quad // QPB) * 2 * H
        if not wrap:
            return [(src, hbm_ref.at[pl.ds(s0 + 2 * _head_of(quad % QPB, 0), 8)], wsem.at[t])]
        na = 8 - 2 * ROT
        return [(src.at[pl.ds(0, na)], hbm_ref.at[pl.ds(s0 + 2 * H - na, na)], wsem.at[t]),
                (src.at[pl.ds(na, 8 - na)], hbm_ref.at[pl.ds(s0, 8 - na)], wsem.at[4 + t])]

    def start_unit(src, hbm_ref, quad, rh, t):
        def go(w):
            parts = unit_parts(src, hbm_ref, quad, t, w)

            def one(c):
                rows = _ads(rh * PART + c * WROWS, WROWS, WROWS)
                for s, d, sem in parts:
                    copy(s.at[:, rows], d.at[:, rows], sem).start()

            _loop(PART // WROWS, one, 2)

        _by_wrap([quad], go)

    def wait_unit(src, hbm_ref, quad, rh, t):
        def go(w):
            rows = _ads(rh * PART, PART, PART)
            for s, d, sem in unit_parts(src, hbm_ref, quad, t, w):
                copy(s.at[:, rows], d.at[:, rows], sem).wait()

        _by_wrap([quad], go)

    def dv_unit(quad, rh):
        return vbuf.at[DVSLOT], dv_hbm, quad, rh, rh

    def dk_unit(quad, rh):
        return vbuf.at[quad % NVSLOT], dk_hbm, quad, rh, 2 + rh


    in_pairs = ((x_hbm, x_s), (go_hbm, go_s), (b1_hbm, b1_s), (b2_hbm, b2_s),
                (wq_hbm, wq), (wo_hbm, wo), (w1_hbm, w1), (w2_hbm, w2))
    out_pairs = ((out_s, out_hbm), (db1_s, db1_hbm), (db2_s, db2_hbm), (dx_s, dx_hbm),
                 (dwq, dwq_hbm), (dwo, dwo_hbm), (dw1, dw1_hbm), (dw2, dw2_hbm))

    def in_copy(n):
        return copy(in_pairs[n][0], in_pairs[n][1], isem.at[n])

    def out_copy(n):
        return copy(out_pairs[n][0], out_pairs[n][1], osem.at[n])

    def start_attn_weights(r):
        qrows = _ads(r * 8, 8, 8)
        for c in range(8):
            qcols = pl.ds(c * 512, 512)
            orows = _ads(r * 64 + c * 8, 8, 8)
            copy(wq_hbm.at[:, qrows, qcols], wq.at[:, qrows, qcols], isem.at[4]).start(priority=0)
            copy(wo_hbm.at[:, orows], wo.at[:, orows], isem.at[5]).start(priority=1)

    def start_mlp_weights(r):
        for c in range(8):
            rows1 = _ads(r * 64 + c * 8, 8, 8)
            copy(w1_hbm.at[rows1], w1.at[rows1], isem.at[6]).start(priority=0)
            if c < 7:
                rows2 = _ads(r * 224 + c * 32, 32, 32)
                copy(w2_hbm.at[rows2], w2.at[rows2], isem.at[7]).start(priority=1)

    def start_attn_grads(r):
        for c in range(8):
            qrows = _ads(r * 16 + (c // 4) * 8, 8, 8)
            qcols = pl.ds((c % 4) * 1024, 1024)
            orows = _ads(r * 128 + c * 16, 16, 16)
            copy(dwq.at[:, qrows, qcols], dwq_hbm.at[:, qrows, qcols], osem.at[4]).start()
            copy(dwo.at[:, orows], dwo_hbm.at[:, orows], osem.at[5]).start()

    def start_mlp_grads(r):
        for c in range(7):
            if c % 2 == 0:
                rows1 = _ads(r * 32 + (c // 2) * 8, 8, 8)
                copy(dw1.at[:, rows1], dw1_hbm.at[:, rows1], osem.at[6]).start()
            rows2 = _ads(r * 112 + c * 16, 16, 16)
            copy(dw2.at[:, rows2], dw2_hbm.at[:, rows2], osem.at[7]).start()


    for n in range(4):
        in_copy(n).start()
    _loop(16, start_attn_weights)
    for ref in (o_all, dq_all, h_all, y_all, dh_all, g_all, da_all, acc_s, ksum_s, ml_s):
        ref[...] = jnp.zeros(ref.shape, F32)
    _loop(8, start_mlp_weights)
    for n in range(6):
        in_copy(n).wait()
    xn_all[...] = _pad_rows(_ln(x_s[...].astype(F32))[0])
    xn_b16 = xn_all[...].astype(BF16)
    for c in range(HD // 1024):
        qc = slice(c * 1024, (c + 1) * 1024)
        q_all[:, qc] = _dot(xn_b16, wq[:, :, qc].reshape(D, 1024)).astype(BF16).astype(F32)
    start_v_head()
    start_kv(0)
    start_kv(1)
    in_copy(6).wait()
    in_copy(7).wait()
    dg_all[...] = _dot_nt(_pad_rows(go_s[...].astype(F32)).astype(BF16), w2[...])
    start_kv(2)

    split_step = (NSITE // B + AHEAD + 2) // 2
    split_pairs = NP + LEAD


    def fwd_half(b, hs):
        site = b * (NSITE // B) + hs
        n = site // 2
        part = n % 4
        jq = hs // 8
        nxt = site + AHEAD

        @pl.when(site == NSITE // B + 2)
        def _():
            wait_unit(*dv_unit(QPB - 1, 0))
            wait_unit(*dv_unit(QPB - 1, 1))

        @pl.when(jnp.logical_and(nxt < NSITE - 1, n != H))
        def _():
            start_kv(nxt, inline=True)

        @pl.when(nxt == NSITE - 1)
        def _():
            start_kv(NSITE - 1, last=True)

        @pl.when(site == NSITE - 3)
        def _():
            wait_v_pairs(NSTEP - 1, 0, 2 * NP - RTAIL // 2)
            start_unit(*dk_unit(QPB - 1, 0))
            start_unit(*dk_unit(QPB - 1, 1))

        @pl.when(site % 2 == 0)
        def _():
            wait_all(*k_dst(n))

            @pl.when(jnp.logical_and(n != split_step, n != NSTEP - 1))
            def _():
                wait_all(*v_dst(n))

            @pl.when(n == split_step)
            def _():
                wait_v_pairs(split_step, split_pairs, 2 * NP)

            @pl.when(n == NSTEP - 1)
            def _():
                wait_v_pairs(NSTEP - 1, 2 * NP - RTAIL // 2, 2 * NP)

        first = part == 0
        heads = []
        for w in range(2):
            u = 2 * (site % 2) + w
            kref = kbuf.at[n % NKSLOT, pl.ds(2 * u, 2)]
            q8 = jnp.broadcast_to(_get_row(q_all, b, _head_lanes(jq, u)), (8, DH)).astype(BF16)
            s = _dot_nt(q8, kref[...].reshape(2 * STEP, DH)) * SCALE
            rows_all[part, pl.ds(4 * jq + u, 1), :] = s[0:1]
            m_old = jnp.where(first, -jnp.inf, ml_s[u, 0])
            m_new = jnp.maximum(m_old, jnp.max(s, axis=1, keepdims=True))
            alpha = jnp.exp(m_old - m_new)
            e = jnp.exp(s - m_new[:, 0:1])
            ml_s[u, 0] = m_new
            ml_s[u, 1] = jnp.where(first, 0.0, ml_s[u, 1] * alpha) + jnp.sum(e, axis=1, keepdims=True)
            e = e.astype(BF16).astype(F32)
            ml_s[u, 2] = jnp.where(first, 0.0, ml_s[u, 2] * alpha) + jnp.sum(e, axis=1, keepdims=True)
            heads.append((u, kref, e, alpha[0:1]))

        for u, kref, e, alpha in heads:
            vref = vbuf.at[(n // 4) % NVSLOT, pl.ds(2 * u, 2), _ads(part * STEP, STEP, STEP)]
            acc = jnp.where(first, 0.0, acc_s[u] * alpha)
            ksum = jnp.where(first, 0.0, ksum_s[u] * alpha)
            for half in range(2):
                ec = e[:, half * STEP:(half + 1) * STEP]
                lhs = jnp.concatenate(
                    [kref[half].T.astype(F32) * ec[0:1], ec, ec], axis=0).astype(BF16)
                acc = acc + _dot(lhs, vref[half])
                for j in range(STEP // DH):
                    ksum = ksum + lhs[0:DH, j * DH:(j + 1) * DH].astype(F32)
            acc_s[u] = acc
            ksum_s[u] = ksum

        @pl.when(part == 3)
        def _():
            for w in range(2):
                u = 2 * (site % 2) + w
                prow = pl.ds(4 * jq + u, 1)
                m = ml_s[u, 0][0:1, 0:1]
                inv_p = 1.0 / ml_s[u, 1][0:1, 0:1]
                for r in range(4):
                    rows_all[r, prow, :] = jnp.exp(rows_all[r, prow, :] - m) * inv_p
                inv = 1.0 / ml_s[u, 2][0:1]
                o8 = acc_s[u, DH:DH + 8, :] * inv
                kbar = jnp.sum(ksum_s[u], axis=1, keepdims=True) * inv
                m_all[4 * jq + u] = ((acc_s[u, 0:DH, :] * inv - kbar * o8[0:1]) * SCALE).astype(BF16)
                _set_row(o_all, b, _head_lanes(jq, u), o8)
                att_s[...] += _dot(o8.astype(BF16), wo_rows(jq, u))


    def mlp_mid(b):
        row = pl.ds(b, 1)
        x2 = x_s[...].astype(F32)
        go2 = go_s[...].astype(F32)
        hh = att_s[...] + jnp.where(b == 0, x2[0:1], x2[1:2])
        go = jnp.where(b == 0, go2[0:1], go2[1:2])
        hn, r1 = _ln(hh)
        y, r2 = _ln(hn)
        a = _dot(y.astype(BF16), w1[...]) + b1_s[...].astype(F32).reshape(1, FF)
        t = jnp.tanh(GELU_C * (a + GELU_A * a * a * a))
        dgelu = 0.5 * (1.0 + t) + 0.5 * a * (1.0 - t * t) * GELU_C * (1.0 + 3.0 * GELU_A * a * a)
        da = dg_all[row, :] * dgelu
        dy = _dot_nt(da.astype(BF16), w1[...])
        dh = go + _ln_bwd(_ln_bwd(dy, y, r2), hn, r1)
        h_all[row, :] = hh[0:1]
        y_all[row, :] = y[0:1]
        g_all[row, :] = (0.5 * a * (1.0 + t))[0:1]
        da_all[row, :] = da[0:1]
        dh_all[row, :] = dh[0:1]

    def mlp_outputs():
        go2 = go_s[...].astype(F32)
        g16 = g_all[...].astype(BF16)
        mlp = _dot(g16, w2[...]) + b2_s[...].astype(F32).reshape(1, D)
        out_s[...] = (h_all[...] + mlp)[0:B].astype(BF16)
        db1_s[...] = (da_all[0:1, :] + da_all[1:2, :]).reshape(FF).astype(BF16)
        db2_s[...] = (go2[0:1] + go2[1:2]).reshape(D).astype(BF16)
        for n in range(3):
            out_copy(n).start()
        go16 = _pad_rows(go2).astype(BF16)
        for c in range(FF // 128):
            dw2[c // 7, (c % 7) * 128:(c % 7 + 1) * 128, :] = _dot_tn(
                g16[:, c * 128:(c + 1) * 128], go16).astype(BF16)
        y16 = y_all[...].astype(BF16)
        da16 = da_all[...].astype(BF16)
        for c in range(D // 128):
            dw1[c // 2, (c % 2) * 128:(c % 2 + 1) * 128, :] = _dot_tn(
                y16[:, c * 128:(c + 1) * 128], da16).astype(BF16)

    def dwo_output():
        o16 = o_all[...].astype(BF16)
        dh16 = dh_all[...].astype(BF16)
        for c in range(HD // 256):
            dwo[c // 4, (c % 4) * 256:(c % 4 + 1) * 256, :] = _dot_tn(
                o16[:, c * 256:(c + 1) * 256], dh16).astype(BF16)


    def bwd_quad(b, jq):
        quad = b * QPB + jq
        slot = quad % NVSLOT
        dh8 = jnp.broadcast_to(dh_all[pl.ds(b, 1), :], (8, D)).astype(BF16)
        for u in range(4):
            cols[0, u] = _dot_nt(dh8, wo_rows(jq, u)).astype(BF16).astype(F32)
            cols[1, u] = jnp.broadcast_to(_get_row(q_all, b, _head_lanes(jq, u)) * SCALE, (8, DH))

        def score_grad(u):
            do8 = cols[0, u].astype(BF16)
            _set_row(dq_all, b, _head_lanes(jq, u), _dot_nt(do8, m_all[4 * jq + u]))
            dp = _dot_nt(do8, vbuf[slot, pl.ds(2 * u, 2)].reshape(S, DH))[0:1]
            prow = pl.ds(4 * jq + u, 1)
            p = jnp.concatenate(
                [rows_all[r, prow, half * STEP:(half + 1) * STEP]
                 for half in range(2) for r in range(4)], axis=1)
            ds = p * (dp - jnp.sum(p * dp, axis=1, keepdims=True))
            for r in range(4):
                for half in range(2):
                    k0 = half * SROWS + r * STEP
                    rows_all[r, pl.ds(H + u, 1), half * STEP:(half + 1) * STEP] = ds[:, k0:k0 + STEP]

        def unit(t):
            kind = t // 2
            rh = t % 2

            @pl.when(jnp.logical_or(t == 1, t == 2))
            def _():
                _loop(2, lambda w: score_grad(2 * (t - 1) + w))

            @pl.when(jnp.logical_and(kind == 0, jq > 0))
            def _():
                wait_unit(*dv_unit(quad - 1, rh))

            @pl.when(jnp.logical_and(kind == 1, quad > 0))
            def _():
                wait_unit(*dk_unit(quad - 1, rh))

            dst = vbuf.at[jnp.where(kind == 0, DVSLOT, slot)]
            row0 = jnp.where(kind == 0, 4 * jq, H)
            for u in range(4):
                col = jnp.broadcast_to(cols[kind, u][0:1], (DH, DH)).T
                for half in range(2):
                    for c in range(PART // CH):
                        rr, l0 = divmod(c * CH, STEP)
                        l0 += half * STEP
                        dst[2 * u + half, _ads(rh * PART + c * CH, CH, CH), :] = _outer_tiles(
                            col, rows_all[2 * rh + rr, pl.ds(row0 + u, 1), l0:l0 + CH])

            @pl.when(jnp.logical_and(quad == 0, t == 0))
            def _():
                wait_v_pairs(split_step, 0, split_pairs - RTAIL // 2)

            @pl.when(jnp.logical_and(quad == 0, t == 1))
            def _():
                wait_v_pairs(split_step, split_pairs - RTAIL // 2, split_pairs)

            @pl.when(kind == 0)
            def _():
                start_unit(*dv_unit(quad, rh))

            @pl.when(jnp.logical_and(kind == 1, quad != QPB - 1))
            def _():
                start_unit(*dk_unit(quad, rh))

        _loop(4, unit)

        @pl.when(quad == QPB)
        def _():
            mlp_outputs()

        @pl.when(quad == QPB + 1)
        def _():
            dwo_output()

    def batch(b):
        att_s[...] = jnp.zeros((8, D), F32)
        _loop(NSITE // B, lambda hs: fwd_half(b, hs))

        @pl.when(b == 0)
        def _():
            start_kv(NSITE // B + AHEAD)

        mlp_mid(b)

        @pl.when(b == 0)
        def _():
            start_kv(NSITE // B + AHEAD + 1)

        _loop(QPB, lambda jq: bwd_quad(b, jq))

    _loop(B, batch)


    dq16 = dq_all[...].astype(BF16)
    xn16 = xn_all[...].astype(BF16)
    for c in range(D // 128):
        for n in range(HD // 1024):
            qc = slice(n * 1024, (n + 1) * 1024)
            dwq[c, :, qc] = _dot_tn(xn16[:, c * 128:(c + 1) * 128], dq16[:, qc]).astype(BF16)
    dxn = _dot_nt(dq16, wq[...].reshape(D, HD))[0:B]
    xn, rstd = _ln(x_s[...].astype(F32))
    dx_s[...] = (dh_all[0:B, :] + _ln_bwd(dxn, xn, rstd)).astype(BF16)
    out_copy(3).start()
    _loop(8, start_attn_grads)
    _loop(8, start_mlp_grads)

    for rh in range(2):
        wait_unit(*dv_unit(NQUAD - 1, rh))
        wait_unit(*dk_unit(NQUAD - 1, rh))
    for n in range(len(out_pairs)):
        out_copy(n).wait()


@jax.jit
def pallas_sequential_preLN__mha_block_cached__mixer_channel_mlp__decode_kernel(
    A_x: jax.Array,
    A_k_cache: jax.Array,
    A_v_cache: jax.Array,
    A_wq: jax.Array,
    A_wo: jax.Array,
    B_x: jax.Array,
    B_w1: jax.Array,
    B_b1: jax.Array,
    B_w2: jax.Array,
    B_b2: jax.Array,
    grad_out: jax.Array,
):
    del B_x
    kv_shape = (2 * B * H, SROWS, DH)
    wq_shape = (4, D // 4, HD)
    wo_shape = (4, HD // 4, D)
    dw1_shape = (2, D // 2, FF)
    dw2_shape = (2, FF // 2, D)
    hbm = pl.BlockSpec(memory_space=pl.ANY)
    out_shape = tuple(
        jax.ShapeDtypeStruct(s, BF16)
        for s in ((B, D), (B, D), kv_shape, kv_shape, wq_shape, wo_shape,
                  dw1_shape, (FF,), dw2_shape, (D,)))
    vm = pltpu.VMEM
    dma = pltpu.SemaphoreType.DMA
    scratch = [
        vm((NKSLOT, 8, STEP, DH), BF16),
        vm((NVSLOT + 1, 8, SROWS, DH), BF16),
        vm(wq_shape, BF16), vm(wo_shape, BF16), vm((D, FF), BF16), vm((FF, D), BF16),
        vm(wq_shape, BF16), vm(wo_shape, BF16), vm(dw1_shape, BF16), vm(dw2_shape, BF16),
        vm((B, D), BF16), vm((B, D), BF16), vm((FF,), BF16), vm((D,), BF16),
        vm((B, D), BF16), vm((B, D), BF16), vm((FF,), BF16), vm((D,), BF16),
        vm((4, H + 8, 2 * STEP), F32), vm((H, DH, DH), BF16),
        vm((4, DH + RP, DH), F32), vm((4, DH, DH), F32), vm((4, 3, 8, DH), F32),
        vm((8, D), F32), vm((2, 4, 8, DH), F32),
        vm((RP, HD), F32), vm((RP, HD), F32), vm((RP, HD), F32),
        vm((RP, D), F32), vm((RP, D), F32), vm((RP, D), F32), vm((RP, D), F32),
        vm((RP, FF), F32), vm((RP, FF), F32), vm((RP, FF), F32),
        dma((NKSLOT,)), dma((NKSLOT,)), dma((8,)), dma((8,)), dma((8,)),
    ]
    out, dx, dk, dv, dwq, dwo, dw1, db1, dw2, db2 = pl.pallas_call(
        _kernel,
        out_shape=out_shape,
        in_specs=[hbm] * 10,
        out_specs=[hbm] * 10,
        scratch_shapes=scratch,
        compiler_params=pltpu.CompilerParams(
            vmem_limit_bytes=124 * 2**20, disable_bounds_checks=True),
    )(A_x.reshape(B, D), A_k_cache.reshape(kv_shape), A_v_cache.reshape(kv_shape),
      A_wq.reshape(wq_shape), A_wo.reshape(wo_shape), B_w1, B_b1, B_w2, B_b2,
      grad_out.reshape(B, D))
    return (out.reshape(A_x.shape), dx.reshape(A_x.shape), dk.reshape(A_k_cache.shape),
            dv.reshape(A_v_cache.shape), dwq.reshape(A_wq.shape), dwo.reshape(A_wo.shape),
            dw1.reshape(B_w1.shape), db1, dw2.reshape(B_w2.shape), db2)
```

```python
import jax
import jax.numpy as jnp
from jax import lax
import jax.experimental.pallas as pl
import jax.experimental.pallas.tpu as pltpu

F32 = jnp.float32
BF16 = jnp.bfloat16

B, H, S, DH = 2, 32, 8192, 128
D, FF = 512, 1792
HD = H * DH
NSTEP = B * H
NSITE = 2 * NSTEP
NQUAD = B * H // 4
QPB = H // 4
SROWS = S // 2
PART = SROWS // 2
STEP = SROWS // 4
AHEAD = 3
NVSLOT = QPB + 1
DVSLOT = NVSLOT
NKSLOT = 3
RROWS = 16
WROWS = 64
NP = STEP // (4 * RROWS)
LEAD = 13
RTAIL = 14
ROT = 3
WRAPQ = 3
CH = 256
RP = 16
SCALE = DH ** -0.5
EPS = 1e-5
GELU_C = 0.7978845608028654
GELU_A = 0.044715

NT = (((1,), (1,)), ((), ()))
TN = (((0,), (0,)), ((), ()))


def _dot(a, b):
    return jnp.dot(a, b, preferred_element_type=F32)


def _dot_nt(a, b):
    return lax.dot_general(a, b, NT, preferred_element_type=F32)


def _dot_tn(a, b):
    return lax.dot_general(a, b, TN, preferred_element_type=F32)


def _ln(x):
    mu = jnp.mean(x, axis=-1, keepdims=True)
    xc = x - mu
    var = jnp.mean(xc * xc, axis=-1, keepdims=True)
    rstd = lax.rsqrt(var + EPS)
    return xc * rstd, rstd


def _ln_bwd(dy, y, rstd):
    m1 = jnp.mean(dy, axis=-1, keepdims=True)
    m2 = jnp.mean(dy * y, axis=-1, keepdims=True)
    return (dy - m1 - y * m2) * rstd


def _pad_rows(x2):
    r = lax.broadcasted_iota(jnp.int32, (RP, x2.shape[1]), 0)
    return jnp.where(r == 0, x2[0:1], jnp.where(r == 1, x2[1:2], 0.0))


def _get_row(ref, b, lanes):
    blk = ref[0:8, lanes]
    return jnp.where(b == 0, blk[0:1], blk[1:2])


def _set_row(ref, b, lanes, val8):
    r = lax.broadcasted_iota(jnp.int32, val8.shape, 0)
    ref[0:8, lanes] = jnp.where(r == b, val8, ref[0:8, lanes])


def _outer_tiles(col, row):
    tiles = [col * row[:, j * DH:(j + 1) * DH] for j in range(row.shape[1] // DH)]
    return jnp.concatenate(tiles, axis=1).astype(BF16).T


def _ads(start, size, align):
    return pl.ds(pl.multiple_of(start, align), size)


def _loop(n, body, unroll=1):
    def wrapped(i, c):
        body(i)
        return c

    lax.fori_loop(0, n, wrapped, 0, unroll=unroll)


def _head_of(jq, u):
    return (4 * (jq + QPB - 1 - WRAPQ) + ROT + u) % H


def _head_lanes(jq, u):
    return _ads(_head_of(jq, u) * DH, DH, DH)


def _by_wrap(quads, fn):
    if not quads:
        fn()
        return

    def rest(w):
        _by_wrap(quads[1:], lambda *ws: fn(w, *ws))

    is_wrap = quads[0] % QPB == WRAPQ
    if isinstance(is_wrap, bool):
        rest(is_wrap)
    else:
        pl.when(is_wrap)(lambda: rest(True))
        pl.when(jnp.logical_not(is_wrap))(lambda: rest(False))


def _kernel(x_hbm, k_hbm, v_hbm, wq_hbm, wo_hbm, w1_hbm, b1_hbm, w2_hbm, b2_hbm, go_hbm,
            out_hbm, dx_hbm, dk_hbm, dv_hbm, dwq_hbm, dwo_hbm, dw1_hbm, db1_hbm, dw2_hbm, db2_hbm,
            kbuf, vbuf, wq, wo, w1, w2, dwq, dwo, dw1, dw2,
            x_s, go_s, b1_s, b2_s, out_s, dx_s, db1_s, db2_s,
            rows_all, m_all, acc_s, ksum_s, ml_s, att_s, cols,
            q_all, o_all, dq_all, xn_all, h_all, y_all, dh_all, g_all, da_all, dg_all,
            ksem, vsem, wsem, isem, osem):
    copy = pltpu.make_async_copy

    def wo_rows(jq, u):
        h = _head_of(jq, u)
        return wo[h // 8, _ads((h % 8) * DH, DH, DH), :]


    def k_dst(n):
        return kbuf.at[n % NKSLOT], ksem.at[n % NKSLOT]

    def v_dst(n):
        rows = _ads((n % 4) * STEP, STEP, STEP)
        return vbuf.at[(n // 4) % NVSLOT, :, rows], vsem.at[n % NKSLOT]

    def reader(hbm_ref, dst_fn, j, wrap):
        n = j // 2
        jq = (n // 4) % QPB
        s0 = (n // H) * 2 * H
        dst, sem = dst_fn(n)
        lo = (j % 2) * (STEP // 2)
        hi = (n % 4) * STEP + lo

        def piece(c, v):
            if wrap:
                u, ns, r, size = 2 * (c % 2) + v, 2, 4 * RROWS * (c // 2), 4 * RROWS
            else:
                u, ns, r, size = 0, 8, RROWS * (2 * c + v), RROWS
            return copy(hbm_ref.at[pl.ds(s0 + 2 * _head_of(jq, u), ns), _ads(hi + r, size, RROWS)],
                        dst.at[pl.ds(2 * u, ns), _ads(lo + r, size, RROWS)], sem)

        return piece

    def start_kv(j, last=False, inline=False):
        def run(n, body):
            if inline:
                for c in range(n):
                    body(c)
            else:
                _loop(n, body)

        def same(w):
            kp, vp = reader(k_hbm, k_dst, j, w), reader(v_hbm, v_dst, j, w)

            def one(c):
                for v in range(2):
                    kp(c, v).start(priority=0)
                    vp(c + LEAD, v).start(priority=1)

            run(NP - LEAD, one)

        def lead(wk, wv=None):
            kp = reader(k_hbm, k_dst, j, wk)
            vp = None if last else reader(v_hbm, v_dst, j + 1, wv)

            def one(c):
                for v in range(2):
                    kp(c + NP - LEAD, v).start(priority=0)
                    if not last:
                        vp(c, v).start(priority=1)

            run(LEAD, one)

        _by_wrap([j // 8], same)
        _by_wrap([j // 8] if last else [j // 8, (j + 1) // 8], lead)

    def start_v_head():
        vp = reader(v_hbm, v_dst, 0, False)

        def one(c):
            for v in range(2):
                vp(c, v).start(priority=v)

        _loop(LEAD, one)

    def wait_all(buf, sem):
        copy(buf, buf, sem).wait()

    def wait_v_pairs(n, c0, c1):
        vp = reader(v_hbm, v_dst, 2 * n, False)

        def one(c):
            for v in range(2):
                vp(c0 + c, v).wait()

        _loop(c1 - c0, one)


    def unit_parts(src, hbm_ref, quad, t, wrap):
        s0 = (quad // QPB) * 2 * H
        if not wrap:
            return [(src, hbm_ref.at[pl.ds(s0 + 2 * _head_of(quad % QPB, 0), 8)], wsem.at[t])]
        na = 8 - 2 * ROT
        return [(src.at[pl.ds(0, na)], hbm_ref.at[pl.ds(s0 + 2 * H - na, na)], wsem.at[t]),
                (src.at[pl.ds(na, 8 - na)], hbm_ref.at[pl.ds(s0, 8 - na)], wsem.at[4 + t])]

    def start_unit(src, hbm_ref, quad, rh, t):
        def go(w):
            parts = unit_parts(src, hbm_ref, quad, t, w)

            def one(c):
                rows = _ads(rh * PART + c * WROWS, WROWS, WROWS)
                for s, d, sem in parts:
                    copy(s.at[:, rows], d.at[:, rows], sem).start()

            _loop(PART // WROWS, one, 2)

        _by_wrap([quad], go)

    def wait_unit(src, hbm_ref, quad, rh, t):
        def go(w):
            rows = _ads(rh * PART, PART, PART)
            for s, d, sem in unit_parts(src, hbm_ref, quad, t, w):
                copy(s.at[:, rows], d.at[:, rows], sem).wait()

        _by_wrap([quad], go)

    def dv_unit(quad, rh):
        return vbuf.at[DVSLOT], dv_hbm, quad, rh, rh

    def dk_unit(quad, rh):
        return vbuf.at[quad % NVSLOT], dk_hbm, quad, rh, 2 + rh


    in_pairs = ((x_hbm, x_s), (go_hbm, go_s), (b1_hbm, b1_s), (b2_hbm, b2_s),
                (wq_hbm, wq), (wo_hbm, wo), (w1_hbm, w1), (w2_hbm, w2))
    out_pairs = ((out_s, out_hbm), (db1_s, db1_hbm), (db2_s, db2_hbm), (dx_s, dx_hbm),
                 (dwq, dwq_hbm), (dwo, dwo_hbm), (dw1, dw1_hbm), (dw2, dw2_hbm))

    def in_copy(n):
        return copy(in_pairs[n][0], in_pairs[n][1], isem.at[n])

    def out_copy(n):
        return copy(out_pairs[n][0], out_pairs[n][1], osem.at[n])

    def start_attn_weights(r):
        qrows = _ads(r * 8, 8, 8)
        for c in range(8):
            qcols = pl.ds(c * 512, 512)
            orows = _ads(((r * 8 + c + 2 * LEAD + 1) % 128) * 8, 8, 8)
            copy(wq_hbm.at[:, qrows, qcols], wq.at[:, qrows, qcols], isem.at[4]).start(priority=0)
            copy(wo_hbm.at[:, orows], wo.at[:, orows], isem.at[5]).start(priority=1)

    def start_mlp_weights(r):
        for c in range(8):
            rows1 = _ads(r * 32 + (c // 2) * 8, 8, 8)
            cols1 = pl.ds((c % 2) * (FF // 2), FF // 2)
            copy(w1_hbm.at[:, rows1, cols1], w1.at[:, rows1, cols1], isem.at[6]).start(priority=0)
            if c < 7:
                rows2 = _ads(r * 112 + c * 16, 16, 16)
                copy(w2_hbm.at[:, rows2], w2.at[:, rows2], isem.at[7]).start(priority=1)

    def start_attn_grads(r):
        for c in range(8):
            qrows = _ads(r * 16 + (c // 4) * 8, 8, 8)
            qcols = pl.ds((c % 4) * 1024, 1024)
            orows = _ads(r * 128 + c * 16, 16, 16)
            copy(dwq.at[:, qrows, qcols], dwq_hbm.at[:, qrows, qcols], osem.at[4]).start()
            copy(dwo.at[:, orows], dwo_hbm.at[:, orows], osem.at[5]).start()

    def start_mlp_grads(r):
        for c in range(7):
            if c % 2 == 0:
                rows1 = _ads(r * 32 + (c // 2) * 8, 8, 8)
                copy(dw1.at[:, rows1], dw1_hbm.at[:, rows1], osem.at[6]).start()
            rows2 = _ads(r * 112 + c * 16, 16, 16)
            copy(dw2.at[:, rows2], dw2_hbm.at[:, rows2], osem.at[7]).start()


    for n in range(4):
        in_copy(n).start()
    _loop(16, start_attn_weights)
    for ref in (o_all, dq_all, h_all, y_all, dh_all, g_all, da_all, acc_s, ksum_s, ml_s):
        ref[...] = jnp.zeros(ref.shape, F32)
    _loop(8, start_mlp_weights)
    for n in range(6):
        in_copy(n).wait()
    xn_all[...] = _pad_rows(_ln(x_s[...].astype(F32))[0])
    xn_b16 = xn_all[...].astype(BF16)
    for c in range(HD // 1024):
        qc = slice(c * 1024, (c + 1) * 1024)
        q_all[:, qc] = _dot(xn_b16, wq[:, :, qc].reshape(D, 1024)).astype(BF16).astype(F32)
    start_v_head()
    start_kv(0)
    start_kv(1)
    in_copy(6).wait()
    in_copy(7).wait()
    dg_all[...] = _dot_nt(_pad_rows(go_s[...].astype(F32)).astype(BF16), w2[...].reshape(FF, D))
    start_kv(2)

    split_step = (NSITE // B + AHEAD + 2) // 2
    split_pairs = NP + LEAD


    def fwd_half(b, hs):
        site = b * (NSITE // B) + hs
        n = site // 2
        part = n % 4
        jq = hs // 8
        nxt = site + AHEAD

        @pl.when(site == NSITE // B + 2)
        def _():
            wait_unit(*dv_unit(QPB - 1, 0))
            wait_unit(*dv_unit(QPB - 1, 1))

        @pl.when(jnp.logical_and(nxt < NSITE - 1, n != H))
        def _():
            start_kv(nxt, inline=True)

        @pl.when(nxt == NSITE - 1)
        def _():
            start_kv(NSITE - 1, last=True)

        @pl.when(site == NSITE - 3)
        def _():
            wait_v_pairs(NSTEP - 1, 0, 2 * NP - RTAIL // 2)
            start_unit(*dk_unit(QPB - 1, 0))
            start_unit(*dk_unit(QPB - 1, 1))

        @pl.when(site % 2 == 0)
        def _():
            wait_all(*k_dst(n))

            @pl.when(jnp.logical_and(n != split_step, n != NSTEP - 1))
            def _():
                wait_all(*v_dst(n))

            @pl.when(n == split_step)
            def _():
                wait_v_pairs(split_step, split_pairs, 2 * NP)

            @pl.when(n == NSTEP - 1)
            def _():
                wait_v_pairs(NSTEP - 1, 2 * NP - RTAIL // 2, 2 * NP)

        first = part == 0
        heads = []
        for w in range(2):
            u = 2 * (site % 2) + w
            kref = kbuf.at[n % NKSLOT, pl.ds(2 * u, 2)]
            q8 = jnp.broadcast_to(_get_row(q_all, b, _head_lanes(jq, u)), (8, DH)).astype(BF16)
            s = _dot_nt(q8, kref[...].reshape(2 * STEP, DH)) * SCALE
            rows_all[part, pl.ds(4 * jq + u, 1), :] = s[0:1]
            m_old = jnp.where(first, -jnp.inf, ml_s[u, 0])
            m_new = jnp.maximum(m_old, jnp.max(s, axis=1, keepdims=True))
            alpha = jnp.exp(m_old - m_new)
            e = jnp.exp(s - m_new[:, 0:1])
            ml_s[u, 0] = m_new
            ml_s[u, 1] = jnp.where(first, 0.0, ml_s[u, 1] * alpha) + jnp.sum(e, axis=1, keepdims=True)
            e = e.astype(BF16).astype(F32)
            ml_s[u, 2] = jnp.where(first, 0.0, ml_s[u, 2] * alpha) + jnp.sum(e, axis=1, keepdims=True)
            heads.append((u, kref, e, alpha[0:1]))

        for u, kref, e, alpha in heads:
            vref = vbuf.at[(n // 4) % NVSLOT, pl.ds(2 * u, 2), _ads(part * STEP, STEP, STEP)]
            acc = jnp.where(first, 0.0, acc_s[u] * alpha)
            ksum = jnp.where(first, 0.0, ksum_s[u] * alpha)
            for half in range(2):
                ec = e[:, half * STEP:(half + 1) * STEP]
                lhs = jnp.concatenate(
                    [kref[half].T.astype(F32) * ec[0:1], ec, ec], axis=0).astype(BF16)
                acc = acc + _dot(lhs, vref[half])
                for j in range(STEP // DH):
                    ksum = ksum + lhs[0:DH, j * DH:(j + 1) * DH].astype(F32)
            acc_s[u] = acc
            ksum_s[u] = ksum

        @pl.when(part == 3)
        def _():
            for w in range(2):
                u = 2 * (site % 2) + w
                prow = pl.ds(4 * jq + u, 1)
                m = ml_s[u, 0][0:1, 0:1]
                inv_p = 1.0 / ml_s[u, 1][0:1, 0:1]
                for r in range(4):
                    rows_all[r, prow, :] = jnp.exp(rows_all[r, prow, :] - m) * inv_p
                inv = 1.0 / ml_s[u, 2][0:1]
                o8 = acc_s[u, DH:DH + 8, :] * inv
                kbar = jnp.sum(ksum_s[u], axis=1, keepdims=True) * inv
                m_all[4 * jq + u] = ((acc_s[u, 0:DH, :] * inv - kbar * o8[0:1]) * SCALE).astype(BF16)
                _set_row(o_all, b, _head_lanes(jq, u), o8)
                att_s[...] += _dot(o8.astype(BF16), wo_rows(jq, u))


    def mlp_mid(b):
        row = pl.ds(b, 1)
        x2 = x_s[...].astype(F32)
        go2 = go_s[...].astype(F32)
        hh = att_s[...] + jnp.where(b == 0, x2[0:1], x2[1:2])
        go = jnp.where(b == 0, go2[0:1], go2[1:2])
        hn, r1 = _ln(hh)
        y, r2 = _ln(hn)
        a = _dot(y.astype(BF16), w1[...].reshape(D, FF)) + b1_s[...].astype(F32).reshape(1, FF)
        t = jnp.tanh(GELU_C * (a + GELU_A * a * a * a))
        dgelu = 0.5 * (1.0 + t) + 0.5 * a * (1.0 - t * t) * GELU_C * (1.0 + 3.0 * GELU_A * a * a)
        da = dg_all[row, :] * dgelu
        dy = _dot_nt(da.astype(BF16), w1[...].reshape(D, FF))
        dh = go + _ln_bwd(_ln_bwd(dy, y, r2), hn, r1)
        h_all[row, :] = hh[0:1]
        y_all[row, :] = y[0:1]
        g_all[row, :] = (0.5 * a * (1.0 + t))[0:1]
        da_all[row, :] = da[0:1]
        dh_all[row, :] = dh[0:1]

    def mlp_outputs():
        go2 = go_s[...].astype(F32)
        g16 = g_all[...].astype(BF16)
        mlp = _dot(g16, w2[...].reshape(FF, D)) + b2_s[...].astype(F32).reshape(1, D)
        out_s[...] = (h_all[...] + mlp)[0:B].astype(BF16)
        db1_s[...] = (da_all[0:1, :] + da_all[1:2, :]).reshape(FF).astype(BF16)
        db2_s[...] = (go2[0:1] + go2[1:2]).reshape(D).astype(BF16)
        for n in range(3):
            out_copy(n).start()
        go16 = _pad_rows(go2).astype(BF16)
        for c in range(FF // 128):
            dw2[c // 7, (c % 7) * 128:(c % 7 + 1) * 128, :] = _dot_tn(
                g16[:, c * 128:(c + 1) * 128], go16).astype(BF16)
        y16 = y_all[...].astype(BF16)
        da16 = da_all[...].astype(BF16)
        for c in range(D // 128):
            dw1[c // 2, (c % 2) * 128:(c % 2 + 1) * 128, :] = _dot_tn(
                y16[:, c * 128:(c + 1) * 128], da16).astype(BF16)

    def dwo_output():
        o16 = o_all[...].astype(BF16)
        dh16 = dh_all[...].astype(BF16)
        for c in range(HD // 256):
            dwo[c // 4, (c % 4) * 256:(c % 4 + 1) * 256, :] = _dot_tn(
                o16[:, c * 256:(c + 1) * 256], dh16).astype(BF16)


    def bwd_quad(b, jq):
        quad = b * QPB + jq
        slot = quad % NVSLOT
        dh8 = jnp.broadcast_to(dh_all[pl.ds(b, 1), :], (8, D)).astype(BF16)
        for u in range(4):
            cols[0, u] = _dot_nt(dh8, wo_rows(jq, u)).astype(BF16).astype(F32)
            cols[1, u] = jnp.broadcast_to(_get_row(q_all, b, _head_lanes(jq, u)) * SCALE, (8, DH))

        def score_grad(u):
            do8 = cols[0, u].astype(BF16)
            _set_row(dq_all, b, _head_lanes(jq, u), _dot_nt(do8, m_all[4 * jq + u]))
            dp = _dot_nt(do8, vbuf[slot, pl.ds(2 * u, 2)].reshape(S, DH))[0:1]
            prow = pl.ds(4 * jq + u, 1)
            p = jnp.concatenate(
                [rows_all[r, prow, half * STEP:(half + 1) * STEP]
                 for half in range(2) for r in range(4)], axis=1)
            ds = p * (dp - jnp.sum(p * dp, axis=1, keepdims=True))
            for r in range(4):
                for half in range(2):
                    k0 = half * SROWS + r * STEP
                    rows_all[r, pl.ds(H + u, 1), half * STEP:(half + 1) * STEP] = ds[:, k0:k0 + STEP]

        def unit(t):
            kind = t // 2
            rh = t % 2

            @pl.when(jnp.logical_or(t == 1, t == 2))
            def _():
                _loop(2, lambda w: score_grad(2 * (t - 1) + w))

            @pl.when(jnp.logical_and(kind == 0, jq > 0))
            def _():
                wait_unit(*dv_unit(quad - 1, rh))

            @pl.when(jnp.logical_and(kind == 1, quad > 0))
            def _():
                wait_unit(*dk_unit(quad - 1, rh))

            dst = vbuf.at[jnp.where(kind == 0, DVSLOT, slot)]
            row0 = jnp.where(kind == 0, 4 * jq, H)
            for u in range(4):
                col = jnp.broadcast_to(cols[kind, u][0:1], (DH, DH)).T
                for half in range(2):
                    for c in range(PART // CH):
                        rr, l0 = divmod(c * CH, STEP)
                        l0 += half * STEP
                        dst[2 * u + half, _ads(rh * PART + c * CH, CH, CH), :] = _outer_tiles(
                            col, rows_all[2 * rh + rr, pl.ds(row0 + u, 1), l0:l0 + CH])

            @pl.when(jnp.logical_and(quad == 0, t == 0))
            def _():
                wait_v_pairs(split_step, 0, split_pairs - RTAIL // 2)

            @pl.when(jnp.logical_and(quad == 0, t == 1))
            def _():
                wait_v_pairs(split_step, split_pairs - RTAIL // 2, split_pairs)

            @pl.when(kind == 0)
            def _():
                start_unit(*dv_unit(quad, rh))

            @pl.when(jnp.logical_and(kind == 1, quad != QPB - 1))
            def _():
                start_unit(*dk_unit(quad, rh))

        _loop(4, unit)

        @pl.when(quad == QPB)
        def _():
            mlp_outputs()

        @pl.when(quad == QPB + 1)
        def _():
            dwo_output()

    def batch(b):
        att_s[...] = jnp.zeros((8, D), F32)
        _loop(NSITE // B, lambda hs: fwd_half(b, hs))

        @pl.when(b == 0)
        def _():
            start_kv(NSITE // B + AHEAD)

        mlp_mid(b)

        @pl.when(b == 0)
        def _():
            start_kv(NSITE // B + AHEAD + 1)

        _loop(QPB, lambda jq: bwd_quad(b, jq))

    _loop(B, batch)


    dq16 = dq_all[...].astype(BF16)
    xn16 = xn_all[...].astype(BF16)
    for c in range(D // 128):
        for n in range(HD // 1024):
            qc = slice(n * 1024, (n + 1) * 1024)
            dwq[c, :, qc] = _dot_tn(xn16[:, c * 128:(c + 1) * 128], dq16[:, qc]).astype(BF16)
    dxn = _dot_nt(dq16, wq[...].reshape(D, HD))[0:B]
    xn, rstd = _ln(x_s[...].astype(F32))
    dx_s[...] = (dh_all[0:B, :] + _ln_bwd(dxn, xn, rstd)).astype(BF16)
    out_copy(3).start()
    _loop(8, start_attn_grads)
    _loop(8, start_mlp_grads)

    for rh in range(2):
        wait_unit(*dv_unit(NQUAD - 1, rh))
        wait_unit(*dk_unit(NQUAD - 1, rh))
    for n in range(len(out_pairs)):
        out_copy(n).wait()


@jax.jit
def pallas_sequential_preLN__mha_block_cached__mixer_channel_mlp__decode_kernel(
    A_x: jax.Array,
    A_k_cache: jax.Array,
    A_v_cache: jax.Array,
    A_wq: jax.Array,
    A_wo: jax.Array,
    B_x: jax.Array,
    B_w1: jax.Array,
    B_b1: jax.Array,
    B_w2: jax.Array,
    B_b2: jax.Array,
    grad_out: jax.Array,
):
    del B_x
    kv_shape = (2 * B * H, SROWS, DH)
    wq_shape = (4, D // 4, HD)
    wo_shape = (4, HD // 4, D)
    w1_shape = (2, D // 2, FF)
    w2_shape = (2, FF // 2, D)
    hbm = pl.BlockSpec(memory_space=pl.ANY)
    out_shape = tuple(
        jax.ShapeDtypeStruct(s, BF16)
        for s in ((B, D), (B, D), kv_shape, kv_shape, wq_shape, wo_shape,
                  w1_shape, (FF,), w2_shape, (D,)))
    vm = pltpu.VMEM
    dma = pltpu.SemaphoreType.DMA
    scratch = [
        vm((NKSLOT, 8, STEP, DH), BF16),
        vm((NVSLOT + 1, 8, SROWS, DH), BF16),
        vm(wq_shape, BF16), vm(wo_shape, BF16), vm(w1_shape, BF16), vm(w2_shape, BF16),
        vm(wq_shape, BF16), vm(wo_shape, BF16), vm(w1_shape, BF16), vm(w2_shape, BF16),
        vm((B, D), BF16), vm((B, D), BF16), vm((FF,), BF16), vm((D,), BF16),
        vm((B, D), BF16), vm((B, D), BF16), vm((FF,), BF16), vm((D,), BF16),
        vm((4, H + 8, 2 * STEP), F32), vm((H, DH, DH), BF16),
        vm((4, DH + RP, DH), F32), vm((4, DH, DH), F32), vm((4, 3, 8, DH), F32),
        vm((8, D), F32), vm((2, 4, 8, DH), F32),
        vm((RP, HD), F32), vm((RP, HD), F32), vm((RP, HD), F32),
        vm((RP, D), F32), vm((RP, D), F32), vm((RP, D), F32), vm((RP, D), F32),
        vm((RP, FF), F32), vm((RP, FF), F32), vm((RP, FF), F32),
        dma((NKSLOT,)), dma((NKSLOT,)), dma((8,)), dma((8,)), dma((8,)),
    ]
    out, dx, dk, dv, dwq, dwo, dw1, db1, dw2, db2 = pl.pallas_call(
        _kernel,
        out_shape=out_shape,
        in_specs=[hbm] * 10,
        out_specs=[hbm] * 10,
        scratch_shapes=scratch,
        compiler_params=pltpu.CompilerParams(
            vmem_limit_bytes=124 * 2**20, disable_bounds_checks=True),
    )(A_x.reshape(B, D), A_k_cache.reshape(kv_shape), A_v_cache.reshape(kv_shape),
      A_wq.reshape(wq_shape), A_wo.reshape(wo_shape), B_w1.reshape(w1_shape), B_b1,
      B_w2.reshape(w2_shape), B_b2, grad_out.reshape(B, D))
    return (out.reshape(A_x.shape), dx.reshape(A_x.shape), dk.reshape(A_k_cache.shape),
            dv.reshape(A_v_cache.shape), dwq.reshape(A_wq.shape), dwo.reshape(A_wo.shape),
            dw1.reshape(B_w1.shape), db1, dw2.reshape(B_w2.shape), db2)
```

```python
import jax
import jax.numpy as jnp
from jax import lax
import jax.experimental.pallas as pl
import jax.experimental.pallas.tpu as pltpu

F32 = jnp.float32
BF16 = jnp.bfloat16

B, H, S, DH = 2, 32, 8192, 128
D, FF = 512, 1792
HD = H * DH
NSTEP = B * H
NSITE = 2 * NSTEP
NQUAD = B * H // 4
QPB = H // 4
SROWS = S // 2
PART = SROWS // 2
STEP = SROWS // 4
AHEAD = 3
NVSLOT = QPB + 1
DVSLOT = NVSLOT
NKSLOT = 3
RROWS = 16
WROWS = 64
NP = STEP // (4 * RROWS)
LEAD = 13
RTAIL = 14
ROT = 3
WRAPQ = 3
CH = 256
RP = 16
SCALE = DH ** -0.5
EPS = 1e-5
GELU_C = 0.7978845608028654
GELU_A = 0.044715

NT = (((1,), (1,)), ((), ()))
TN = (((0,), (0,)), ((), ()))


def _dot(a, b):
    return jnp.dot(a, b, preferred_element_type=F32)


def _dot_nt(a, b):
    return lax.dot_general(a, b, NT, preferred_element_type=F32)


def _dot_tn(a, b):
    return lax.dot_general(a, b, TN, preferred_element_type=F32)


def _ln(x):
    mu = jnp.mean(x, axis=-1, keepdims=True)
    xc = x - mu
    var = jnp.mean(xc * xc, axis=-1, keepdims=True)
    rstd = lax.rsqrt(var + EPS)
    return xc * rstd, rstd


def _ln_bwd(dy, y, rstd):
    m1 = jnp.mean(dy, axis=-1, keepdims=True)
    m2 = jnp.mean(dy * y, axis=-1, keepdims=True)
    return (dy - m1 - y * m2) * rstd


def _pad_rows(x2):
    r = lax.broadcasted_iota(jnp.int32, (RP, x2.shape[1]), 0)
    return jnp.where(r == 0, x2[0:1], jnp.where(r == 1, x2[1:2], 0.0))


def _get_row(ref, b, lanes):
    blk = ref[0:8, lanes]
    return jnp.where(b == 0, blk[0:1], blk[1:2])


def _set_row(ref, b, lanes, val8):
    r = lax.broadcasted_iota(jnp.int32, val8.shape, 0)
    ref[0:8, lanes] = jnp.where(r == b, val8, ref[0:8, lanes])


def _outer_tiles(col, row):
    tiles = [col * row[:, j * DH:(j + 1) * DH] for j in range(row.shape[1] // DH)]
    return jnp.concatenate(tiles, axis=1).astype(BF16).T


def _ads(start, size, align):
    return pl.ds(pl.multiple_of(start, align), size)


def _loop(n, body, unroll=1):
    def wrapped(i, c):
        body(i)
        return c

    lax.fori_loop(0, n, wrapped, 0, unroll=unroll)


def _head_of(jq, u):
    return (4 * (jq + QPB - 1 - WRAPQ) + ROT + u) % H


def _head_lanes(jq, u):
    return _ads(_head_of(jq, u) * DH, DH, DH)


def _by_wrap(quads, fn):
    if not quads:
        fn()
        return

    def rest(w):
        _by_wrap(quads[1:], lambda *ws: fn(w, *ws))

    is_wrap = quads[0] % QPB == WRAPQ
    if isinstance(is_wrap, bool):
        rest(is_wrap)
    else:
        pl.when(is_wrap)(lambda: rest(True))
        pl.when(jnp.logical_not(is_wrap))(lambda: rest(False))


def _kernel(x_hbm, k_hbm, v_hbm, wq_hbm, wo_hbm, w1_hbm, b1_hbm, w2_hbm, b2_hbm, go_hbm,
            out_hbm, dx_hbm, dk_hbm, dv_hbm, dwq_hbm, dwo_hbm, dw1_hbm, db1_hbm, dw2_hbm, db2_hbm,
            kbuf, vbuf, wq, wo, w1, w2, dwq, dwo, dw1, dw2,
            x_s, go_s, b1_s, b2_s, out_s, dx_s, db1_s, db2_s,
            rows_all, m_all, acc_s, ksum_s, ml_s, att_s, cols,
            q_all, o_all, dq_all, xn_all, h_all, y_all, dh_all, g_all, da_all, dg_all,
            ksem, vsem, wsem, isem, osem):
    copy = pltpu.make_async_copy

    def wo_rows(jq, u):
        h = _head_of(jq, u)
        return wo[h // 8, pl.ds((h % 8) * 16, 16)].reshape(DH, D)


    def k_dst(n):
        return kbuf.at[n % NKSLOT], ksem.at[n % NKSLOT]

    def v_dst(n):
        rows = _ads((n % 4) * STEP, STEP, STEP)
        return vbuf.at[(n // 4) % NVSLOT, :, rows], vsem.at[n % NKSLOT]

    def reader(hbm_ref, dst_fn, j, wrap):
        n = j // 2
        jq = (n // 4) % QPB
        s0 = (n // H) * 2 * H
        dst, sem = dst_fn(n)
        lo = (j % 2) * (STEP // 2)
        hi = (n % 4) * STEP + lo

        def piece(c, v):
            if wrap:
                u, ns, r, size = 2 * (c % 2) + v, 2, 4 * RROWS * (c // 2), 4 * RROWS
            else:
                u, ns, r, size = 0, 8, RROWS * (2 * c + v), RROWS
            return copy(hbm_ref.at[pl.ds(s0 + 2 * _head_of(jq, u), ns), _ads(hi + r, size, RROWS)],
                        dst.at[pl.ds(2 * u, ns), _ads(lo + r, size, RROWS)], sem)

        return piece

    def start_kv(j, last=False, inline=False):
        def run(n, body):
            if inline:
                for c in range(n):
                    body(c)
            else:
                _loop(n, body)

        def same(w):
            kp, vp = reader(k_hbm, k_dst, j, w), reader(v_hbm, v_dst, j, w)

            def one(c):
                for v in range(2):
                    kp(c, v).start(priority=0)
                    vp(c + LEAD, v).start(priority=1)

            run(NP - LEAD, one)

        def lead(wk, wv=None):
            kp = reader(k_hbm, k_dst, j, wk)
            vp = None if last else reader(v_hbm, v_dst, j + 1, wv)

            def one(c):
                for v in range(2):
                    kp(c + NP - LEAD, v).start(priority=0)
                    if not last:
                        vp(c, v).start(priority=1)

            run(LEAD, one)

        _by_wrap([j // 8], same)
        _by_wrap([j // 8] if last else [j // 8, (j + 1) // 8], lead)

    def start_v_head():
        vp = reader(v_hbm, v_dst, 0, False)

        def one(c):
            for v in range(2):
                vp(c, v).start(priority=v)

        _loop(LEAD, one)

    def wait_all(buf, sem):
        copy(buf, buf, sem).wait()

    def wait_v_pairs(n, c0, c1):
        vp = reader(v_hbm, v_dst, 2 * n, False)

        def one(c):
            for v in range(2):
                vp(c0 + c, v).wait()

        _loop(c1 - c0, one)


    def unit_parts(src, hbm_ref, quad, t, wrap):
        s0 = (quad // QPB) * 2 * H
        if not wrap:
            return [(src, hbm_ref.at[pl.ds(s0 + 2 * _head_of(quad % QPB, 0), 8)], wsem.at[t])]
        na = 8 - 2 * ROT
        return [(src.at[pl.ds(0, na)], hbm_ref.at[pl.ds(s0 + 2 * H - na, na)], wsem.at[t]),
                (src.at[pl.ds(na, 8 - na)], hbm_ref.at[pl.ds(s0, 8 - na)], wsem.at[4 + t])]

    def start_unit(src, hbm_ref, quad, rh, t):
        def go(w):
            parts = unit_parts(src, hbm_ref, quad, t, w)

            def one(c):
                rows = _ads(rh * PART + c * WROWS, WROWS, WROWS)
                for s, d, sem in parts:
                    copy(s.at[:, rows], d.at[:, rows], sem).start()

            _loop(PART // WROWS, one, 2)

        _by_wrap([quad], go)

    def wait_unit(src, hbm_ref, quad, rh, t):
        def go(w):
            rows = _ads(rh * PART, PART, PART)
            for s, d, sem in unit_parts(src, hbm_ref, quad, t, w):
                copy(s.at[:, rows], d.at[:, rows], sem).wait()

        _by_wrap([quad], go)

    def dv_unit(quad, rh):
        return vbuf.at[DVSLOT], dv_hbm, quad, rh, rh

    def dk_unit(quad, rh):
        return vbuf.at[quad % NVSLOT], dk_hbm, quad, rh, 2 + rh


    in_pairs = ((x_hbm, x_s), (go_hbm, go_s), (b1_hbm, b1_s), (b2_hbm, b2_s),
                (wq_hbm, wq), (wo_hbm, wo), (w1_hbm, w1), (w2_hbm, w2))
    out_pairs = ((out_s, out_hbm), (db1_s, db1_hbm), (db2_s, db2_hbm), (dx_s, dx_hbm),
                 (dwq, dwq_hbm), (dwo, dwo_hbm), (dw1, dw1_hbm), (dw2, dw2_hbm))

    def in_copy(n):
        return copy(in_pairs[n][0], in_pairs[n][1], isem.at[n])

    def out_copy(n):
        return copy(out_pairs[n][0], out_pairs[n][1], osem.at[n])

    def start_attn_weights(r):
        for c in range(8):
            qcols = pl.ds(c * 512, 512)
            g = (r * 8 + c + 2 * LEAD + 1) % 128
            copy(wq_hbm.at[:, r, :, qcols], wq.at[:, r, :, qcols], isem.at[4]).start(priority=0)
            copy(wo_hbm.at[:, g], wo.at[:, g], isem.at[5]).start(priority=1)

    def start_mlp_weights(r):
        for c in range(8):
            g = r * 4 + c // 2
            cols1 = pl.ds((c % 2) * (FF // 2), FF // 2)
            copy(w1_hbm.at[:, g, :, cols1], w1.at[:, g, :, cols1], isem.at[6]).start(priority=0)
            if c < 7:
                rows2 = _ads(r * 112 + c * 16, 16, 16)
                copy(w2_hbm.at[:, rows2], w2.at[:, rows2], isem.at[7]).start(priority=1)

    def start_attn_grads(r):
        for c in range(8):
            g = 2 * r + c // 4
            qcols = pl.ds((c % 4) * 1024, 1024)
            orows = _ads(r * 128 + c * 16, 16, 16)
            copy(dwq.at[:, g, :, qcols], dwq_hbm.at[:, g, :, qcols], osem.at[4]).start()
            copy(dwo.at[:, orows], dwo_hbm.at[:, orows], osem.at[5]).start()

    def start_mlp_grads(r):
        for c in range(7):
            if c % 2 == 0:
                g = r * 4 + c // 2
                copy(dw1.at[:, g], dw1_hbm.at[:, g], osem.at[6]).start()
            rows2 = _ads(r * 112 + c * 16, 16, 16)
            copy(dw2.at[:, rows2], dw2_hbm.at[:, rows2], osem.at[7]).start()


    for n in range(4):
        in_copy(n).start()
    _loop(16, start_attn_weights)
    for ref in (o_all, dq_all, h_all, y_all, dh_all, g_all, da_all, acc_s, ksum_s, ml_s):
        ref[...] = jnp.zeros(ref.shape, F32)
    _loop(8, start_mlp_weights)
    for n in range(6):
        in_copy(n).wait()
    xn_all[...] = _pad_rows(_ln(x_s[...].astype(F32))[0])
    xn_b16 = xn_all[...].astype(BF16)
    for c in range(HD // 1024):
        qc = slice(c * 1024, (c + 1) * 1024)
        q_all[:, qc] = _dot(xn_b16, wq[:, :, :, qc].reshape(D, 1024)).astype(BF16).astype(F32)
    start_v_head()
    start_kv(0)
    start_kv(1)
    in_copy(6).wait()
    in_copy(7).wait()
    dg_all[...] = _dot_nt(_pad_rows(go_s[...].astype(F32)).astype(BF16), w2[...].reshape(FF, D))
    start_kv(2)

    split_step = (NSITE // B + AHEAD + 2) // 2
    split_pairs = NP + LEAD


    def fwd_half(b, hs):
        site = b * (NSITE // B) + hs
        n = site // 2
        part = n % 4
        jq = hs // 8
        nxt = site + AHEAD

        @pl.when(site == NSITE // B + 2)
        def _():
            wait_unit(*dv_unit(QPB - 1, 0))
            wait_unit(*dv_unit(QPB - 1, 1))

        @pl.when(jnp.logical_and(nxt < NSITE - 1, n != H))
        def _():
            start_kv(nxt, inline=True)

        @pl.when(nxt == NSITE - 1)
        def _():
            start_kv(NSITE - 1, last=True)

        @pl.when(site == NSITE - 3)
        def _():
            wait_v_pairs(NSTEP - 1, 0, 2 * NP - RTAIL // 2)
            start_unit(*dk_unit(QPB - 1, 0))
            start_unit(*dk_unit(QPB - 1, 1))

        @pl.when(site % 2 == 0)
        def _():
            wait_all(*k_dst(n))

            @pl.when(jnp.logical_and(n != split_step, n != NSTEP - 1))
            def _():
                wait_all(*v_dst(n))

            @pl.when(n == split_step)
            def _():
                wait_v_pairs(split_step, split_pairs, 2 * NP)

            @pl.when(n == NSTEP - 1)
            def _():
                wait_v_pairs(NSTEP - 1, 2 * NP - RTAIL // 2, 2 * NP)

        first = part == 0
        heads = []
        for w in range(2):
            u = 2 * (site % 2) + w
            kref = kbuf.at[n % NKSLOT, pl.ds(2 * u, 2)]
            q8 = jnp.broadcast_to(_get_row(q_all, b, _head_lanes(jq, u)), (8, DH)).astype(BF16)
            s = _dot_nt(q8, kref[...].reshape(2 * STEP, DH)) * SCALE
            rows_all[part, pl.ds(4 * jq + u, 1), :] = s[0:1]
            m_old = jnp.where(first, -jnp.inf, ml_s[u, 0])
            m_new = jnp.maximum(m_old, jnp.max(s, axis=1, keepdims=True))
            alpha = jnp.exp(m_old - m_new)
            e = jnp.exp(s - m_new[:, 0:1])
            ml_s[u, 0] = m_new
            ml_s[u, 1] = jnp.where(first, 0.0, ml_s[u, 1] * alpha) + jnp.sum(e, axis=1, keepdims=True)
            e = e.astype(BF16).astype(F32)
            ml_s[u, 2] = jnp.where(first, 0.0, ml_s[u, 2] * alpha) + jnp.sum(e, axis=1, keepdims=True)
            heads.append((u, kref, e, alpha[0:1]))

        for u, kref, e, alpha in heads:
            vref = vbuf.at[(n // 4) % NVSLOT, pl.ds(2 * u, 2), _ads(part * STEP, STEP, STEP)]
            acc = jnp.where(first, 0.0, acc_s[u] * alpha)
            ksum = jnp.where(first, 0.0, ksum_s[u] * alpha)
            for half in range(2):
                ec = e[:, half * STEP:(half + 1) * STEP]
                lhs = jnp.concatenate(
                    [kref[half].T.astype(F32) * ec[0:1], ec, ec], axis=0).astype(BF16)
                acc = acc + _dot(lhs, vref[half])
                for j in range(STEP // DH):
                    ksum = ksum + lhs[0:DH, j * DH:(j + 1) * DH].astype(F32)
            acc_s[u] = acc
            ksum_s[u] = ksum

        @pl.when(part == 3)
        def _():
            for w in range(2):
                u = 2 * (site % 2) + w
                prow = pl.ds(4 * jq + u, 1)
                m = ml_s[u, 0][0:1, 0:1]
                inv_p = 1.0 / ml_s[u, 1][0:1, 0:1]
                for r in range(4):
                    rows_all[r, prow, :] = jnp.exp(rows_all[r, prow, :] - m) * inv_p
                inv = 1.0 / ml_s[u, 2][0:1]
                o8 = acc_s[u, DH:DH + 8, :] * inv
                kbar = jnp.sum(ksum_s[u], axis=1, keepdims=True) * inv
                m_all[4 * jq + u] = ((acc_s[u, 0:DH, :] * inv - kbar * o8[0:1]) * SCALE).astype(BF16)
                _set_row(o_all, b, _head_lanes(jq, u), o8)
                att_s[...] += _dot(o8.astype(BF16), wo_rows(jq, u))


    def mlp_mid(b):
        row = pl.ds(b, 1)
        x2 = x_s[...].astype(F32)
        go2 = go_s[...].astype(F32)
        hh = att_s[...] + jnp.where(b == 0, x2[0:1], x2[1:2])
        go = jnp.where(b == 0, go2[0:1], go2[1:2])
        hn, r1 = _ln(hh)
        y, r2 = _ln(hn)
        a = _dot(y.astype(BF16), w1[...].reshape(D, FF)) + b1_s[...].astype(F32).reshape(1, FF)
        t = jnp.tanh(GELU_C * (a + GELU_A * a * a * a))
        dgelu = 0.5 * (1.0 + t) + 0.5 * a * (1.0 - t * t) * GELU_C * (1.0 + 3.0 * GELU_A * a * a)
        da = dg_all[row, :] * dgelu
        dy = _dot_nt(da.astype(BF16), w1[...].reshape(D, FF))
        dh = go + _ln_bwd(_ln_bwd(dy, y, r2), hn, r1)
        h_all[row, :] = hh[0:1]
        y_all[row, :] = y[0:1]
        g_all[row, :] = (0.5 * a * (1.0 + t))[0:1]
        da_all[row, :] = da[0:1]
        dh_all[row, :] = dh[0:1]

    def mlp_outputs():
        go2 = go_s[...].astype(F32)
        g16 = g_all[...].astype(BF16)
        mlp = _dot(g16, w2[...].reshape(FF, D)) + b2_s[...].astype(F32).reshape(1, D)
        out_s[...] = (h_all[...] + mlp)[0:B].astype(BF16)
        db1_s[...] = (da_all[0:1, :] + da_all[1:2, :]).reshape(FF).astype(BF16)
        db2_s[...] = (go2[0:1] + go2[1:2]).reshape(D).astype(BF16)
        for n in range(3):
            out_copy(n).start()
        go16 = _pad_rows(go2).astype(BF16)
        for c in range(FF // 128):
            dw2[c // 7, (c % 7) * 128:(c % 7 + 1) * 128, :] = _dot_tn(
                g16[:, c * 128:(c + 1) * 128], go16).astype(BF16)
        y16 = y_all[...].astype(BF16)
        da16 = da_all[...].astype(BF16)
        for c in range(D // 128):
            blk = _dot_tn(y16[:, c * 128:(c + 1) * 128], da16)
            dw1[c // 2, (c % 2) * 16:(c % 2 + 1) * 16] = blk.reshape(16, 8, FF).astype(BF16)

    def dwo_output():
        o16 = o_all[...].astype(BF16)
        dh16 = dh_all[...].astype(BF16)
        for c in range(HD // 256):
            dwo[c // 4, (c % 4) * 256:(c % 4 + 1) * 256, :] = _dot_tn(
                o16[:, c * 256:(c + 1) * 256], dh16).astype(BF16)


    def bwd_quad(b, jq):
        quad = b * QPB + jq
        slot = quad % NVSLOT
        dh8 = jnp.broadcast_to(dh_all[pl.ds(b, 1), :], (8, D)).astype(BF16)
        for u in range(4):
            cols[0, u] = _dot_nt(dh8, wo_rows(jq, u)).astype(BF16).astype(F32)
            cols[1, u] = jnp.broadcast_to(_get_row(q_all, b, _head_lanes(jq, u)) * SCALE, (8, DH))

        def score_grad(u):
            do8 = cols[0, u].astype(BF16)
            _set_row(dq_all, b, _head_lanes(jq, u), _dot_nt(do8, m_all[4 * jq + u]))
            dp = _dot_nt(do8, vbuf[slot, pl.ds(2 * u, 2)].reshape(S, DH))[0:1]
            prow = pl.ds(4 * jq + u, 1)
            p = jnp.concatenate(
                [rows_all[r, prow, half * STEP:(half + 1) * STEP]
                 for half in range(2) for r in range(4)], axis=1)
            ds = p * (dp - jnp.sum(p * dp, axis=1, keepdims=True))
            for r in range(4):
                for half in range(2):
                    k0 = half * SROWS + r * STEP
                    rows_all[r, pl.ds(H + u, 1), half * STEP:(half + 1) * STEP] = ds[:, k0:k0 + STEP]

        def unit(t):
            kind = t // 2
            rh = t % 2

            @pl.when(jnp.logical_or(t == 1, t == 2))
            def _():
                _loop(2, lambda w: score_grad(2 * (t - 1) + w))

            @pl.when(jnp.logical_and(kind == 0, jq > 0))
            def _():
                wait_unit(*dv_unit(quad - 1, rh))

            @pl.when(jnp.logical_and(kind == 1, quad > 0))
            def _():
                wait_unit(*dk_unit(quad - 1, rh))

            dst = vbuf.at[jnp.where(kind == 0, DVSLOT, slot)]
            row0 = jnp.where(kind == 0, 4 * jq, H)
            for u in range(4):
                col = jnp.broadcast_to(cols[kind, u][0:1], (DH, DH)).T
                for half in range(2):
                    for c in range(PART // CH):
                        rr, l0 = divmod(c * CH, STEP)
                        l0 += half * STEP
                        dst[2 * u + half, _ads(rh * PART + c * CH, CH, CH), :] = _outer_tiles(
                            col, rows_all[2 * rh + rr, pl.ds(row0 + u, 1), l0:l0 + CH])

            @pl.when(jnp.logical_and(quad == 0, t == 0))
            def _():
                wait_v_pairs(split_step, 0, split_pairs - RTAIL // 2)

            @pl.when(jnp.logical_and(quad == 0, t == 1))
            def _():
                wait_v_pairs(split_step, split_pairs - RTAIL // 2, split_pairs)

            @pl.when(kind == 0)
            def _():
                start_unit(*dv_unit(quad, rh))

            @pl.when(jnp.logical_and(kind == 1, quad != QPB - 1))
            def _():
                start_unit(*dk_unit(quad, rh))

        _loop(4, unit)

        @pl.when(quad == QPB)
        def _():
            mlp_outputs()

        @pl.when(quad == QPB + 1)
        def _():
            dwo_output()

    def batch(b):
        att_s[...] = jnp.zeros((8, D), F32)
        _loop(NSITE // B, lambda hs: fwd_half(b, hs))

        @pl.when(b == 0)
        def _():
            start_kv(NSITE // B + AHEAD)

        mlp_mid(b)

        @pl.when(b == 0)
        def _():
            start_kv(NSITE // B + AHEAD + 1)

        _loop(QPB, lambda jq: bwd_quad(b, jq))

    _loop(B, batch)


    dq16 = dq_all[...].astype(BF16)
    xn16 = xn_all[...].astype(BF16)
    for c in range(D // 128):
        for n in range(HD // 1024):
            qc = slice(n * 1024, (n + 1) * 1024)
            blk = _dot_tn(xn16[:, c * 128:(c + 1) * 128], dq16[:, qc])
            dwq[c, :, :, qc] = blk.reshape(16, 8, 1024).astype(BF16)
    dxn = _dot_nt(dq16, wq[...].reshape(D, HD))[0:B]
    xn, rstd = _ln(x_s[...].astype(F32))
    dx_s[...] = (dh_all[0:B, :] + _ln_bwd(dxn, xn, rstd)).astype(BF16)
    out_copy(3).start()
    _loop(8, start_attn_grads)
    _loop(8, start_mlp_grads)

    for rh in range(2):
        wait_unit(*dv_unit(NQUAD - 1, rh))
        wait_unit(*dk_unit(NQUAD - 1, rh))
    for n in range(len(out_pairs)):
        out_copy(n).wait()


@jax.jit
def pallas_sequential_preLN__mha_block_cached__mixer_channel_mlp__decode_kernel(
    A_x: jax.Array,
    A_k_cache: jax.Array,
    A_v_cache: jax.Array,
    A_wq: jax.Array,
    A_wo: jax.Array,
    B_x: jax.Array,
    B_w1: jax.Array,
    B_b1: jax.Array,
    B_w2: jax.Array,
    B_b2: jax.Array,
    grad_out: jax.Array,
):
    del B_x
    kv_shape = (2 * B * H, SROWS, DH)
    wq_shape = (4, D // 32, 8, HD)
    wo_shape = (4, HD // 32, 8, D)
    dwo_shape = (4, HD // 4, D)
    w1_shape = (2, D // 16, 8, FF)
    w2_shape = (2, FF // 2, D)
    hbm = pl.BlockSpec(memory_space=pl.ANY)
    out_shape = tuple(
        jax.ShapeDtypeStruct(s, BF16)
        for s in ((B, D), (B, D), kv_shape, kv_shape, wq_shape, dwo_shape,
                  w1_shape, (FF,), w2_shape, (D,)))
    vm = pltpu.VMEM
    dma = pltpu.SemaphoreType.DMA
    scratch = [
        vm((NKSLOT, 8, STEP, DH), BF16),
        vm((NVSLOT + 1, 8, SROWS, DH), BF16),
        vm(wq_shape, BF16), vm(wo_shape, BF16), vm(w1_shape, BF16), vm(w2_shape, BF16),
        vm(wq_shape, BF16), vm(dwo_shape, BF16), vm(w1_shape, BF16), vm(w2_shape, BF16),
        vm((B, D), BF16), vm((B, D), BF16), vm((FF,), BF16), vm((D,), BF16),
        vm((B, D), BF16), vm((B, D), BF16), vm((FF,), BF16), vm((D,), BF16),
        vm((4, H + 8, 2 * STEP), F32), vm((H, DH, DH), BF16),
        vm((4, DH + RP, DH), F32), vm((4, DH, DH), F32), vm((4, 3, 8, DH), F32),
        vm((8, D), F32), vm((2, 4, 8, DH), F32),
        vm((RP, HD), F32), vm((RP, HD), F32), vm((RP, HD), F32),
        vm((RP, D), F32), vm((RP, D), F32), vm((RP, D), F32), vm((RP, D), F32),
        vm((RP, FF), F32), vm((RP, FF), F32), vm((RP, FF), F32),
        dma((NKSLOT,)), dma((NKSLOT,)), dma((8,)), dma((8,)), dma((8,)),
    ]
    out, dx, dk, dv, dwq, dwo, dw1, db1, dw2, db2 = pl.pallas_call(
        _kernel,
        out_shape=out_shape,
        in_specs=[hbm] * 10,
        out_specs=[hbm] * 10,
        scratch_shapes=scratch,
        compiler_params=pltpu.CompilerParams(
            vmem_limit_bytes=124 * 2**20, disable_bounds_checks=True),
    )(A_x.reshape(B, D), A_k_cache.reshape(kv_shape), A_v_cache.reshape(kv_shape),
      A_wq.reshape(wq_shape), A_wo.reshape(wo_shape), B_w1.reshape(w1_shape), B_b1,
      B_w2.reshape(w2_shape), B_b2, grad_out.reshape(B, D))
    return (out.reshape(A_x.shape), dx.reshape(A_x.shape), dk.reshape(A_k_cache.shape),
            dv.reshape(A_v_cache.shape), dwq.reshape(A_wq.shape), dwo.reshape(A_wo.shape),
            dw1.reshape(B_w1.shape), db1, dw2.reshape(B_w2.shape), db2)
```
